```python
import jax
import jax.numpy as jnp

def _softmax(x, axis=-1):
    return jax.nn.softmax(x, axis=axis)
def _gelu(x):
    return jax.nn.gelu(x, approximate=True)
def _silu(x):
    return jax.nn.silu(x)
def _sigmoid(x):
    return jax.nn.sigmoid(x)
def _layernorm(x, axis=-1, eps=1e-5):
    m = jnp.mean(x, axis=axis, keepdims=True)
    v = jnp.var(x, axis=axis, keepdims=True)
    return (x - m) / jnp.sqrt(v + eps)
def _scatter_add(tgt, idx, src, axis=0):
    return tgt.at[idx].add(src)
def _segment_sum(src, seg, n):
    return jax.ops.segment_sum(src, seg, n)
class _Rng:
    def __init__(self, key):
        self._k = key
    def _next(self):
        self._k, sub = jax.random.split(self._k)
        return sub
    def normal(self, shape):
        return jax.random.normal(self._next(), shape, dtype=jnp.bfloat16)
    def randint(self, lo, hi, shape):
        return jax.random.randint(self._next(), shape, lo, hi, dtype=jnp.int32)
    def uniform(self, shape, lo=0.0, hi=1.0):
        return jax.random.uniform(self._next(), shape, jnp.bfloat16, lo, hi)
    def permutation(self, n):
        return jax.random.permutation(self._next(), n)


kernel_name = 'recurrent_scan__sliding_local_dilated__moe_arch_mod__prompt'

def setup_inputs():
    _rng = _Rng(jax.random.key(int.from_bytes(__import__("os").urandom(4), "little")))
    _w = (lambda a: (lambda t: t.astype(jnp.bfloat16) if jnp.issubdtype(t.dtype, jnp.floating) else t)(jnp.asarray(a)))
    def _A_setup():
        B, S, D = 1, 2048, 640
        return {
            "x": _w((lambda *s: _rng.normal(s) * 0.05)(B, S, D)),
            "wqkv": _w((lambda *s: _rng.normal(s) * 0.05)(D, 3 * D)),
            "wo": _w((lambda *s: _rng.normal(s) * 0.05)(D, D)),
        }
    _A_in = _A_setup()

    def _B_setup():
        B, S, D, F, C = 1, 2048, 640, 1728, 2
        return {
            "x": _w((lambda *s: _rng.normal(s) * 0.05)(B, S, D)),
            "w_r": _w((lambda *s: _rng.normal(s) * 0.05)(D)),
            "w_gate": _w((lambda *s: _rng.normal(s) * 0.05)(D, F)),
            "w_up": _w((lambda *s: _rng.normal(s) * 0.05)(D, F)),
            "w_down": _w((lambda *s: _rng.normal(s) * 0.05)(F, D)),
        }
    _B_in = _B_setup()

    return {
        "A_x": _A_in["x"],
        "A_wqkv": _A_in["wqkv"],
        "A_wo": _A_in["wo"],
        "B_x": _B_in["x"],
        "B_w_r": _B_in["w_r"],
        "B_w_gate": _B_in["w_gate"],
        "B_w_up": _B_in["w_up"],
        "B_w_down": _B_in["w_down"],
    }

def reference(A_x, A_wqkv, A_wo, B_x, B_w_r, B_w_gate, B_w_up, B_w_down):
    def _A_ref(x, wqkv, wo):
        B, S, D = x.shape
        H = 32; Dh = D // H
        W, dil = 8, 2
        qkv = (lambda x, *d: x.transpose(*d))((x @ wqkv).reshape(B, S, 3, H, Dh), 2, 0, 3, 1, 4)
        q, k, v = qkv[0], qkv[1], qkv[2]
        scale = Dh ** -0.5
        pos = jnp.arange(S)
        off = jnp.arange(W) * dil
        idx = pos[:, None] - off[None, :]
        mask = idx >= 0
        idx_c = jnp.where(mask, idx, 0).reshape(-1)
        kg = k[:, :, idx_c, :].reshape(B, H, S, W, Dh)
        vg = v[:, :, idx_c, :].reshape(B, H, S, W, Dh)
        logits = jnp.einsum("bhsd,bhswd->bhsw", q, kg) * scale
        logits = jnp.where(mask[None, None, :, :], logits, -1e9)
        attn = _softmax(logits, axis=-1)
        o = jnp.einsum("bhsw,bhswd->bhsd", attn, vg)
        return (lambda x, *d: x.transpose(*d))(o, 0, 2, 1, 3).reshape(B, S, D) @ wo

    def _B_ref(x, w_r, w_gate, w_up, w_down):
        B, S, D = x.shape
        C = 2
        r = x @ w_r
        idx = jnp.argsort(-r, axis=-1)[:, :C]
        idx_e = jnp.repeat(idx.reshape(B, C, 1), D, axis=2)
        x_sel = jnp.take_along_axis(x, idx_e, axis=1)
        g = _silu(x_sel @ w_gate)
        u = x_sel @ w_up
        y = (g * u) @ w_down
        r_sel = _sigmoid(jnp.take_along_axis(r, idx, axis=1))
        y = y * r_sel.reshape(B, C, 1)
        b_off = (jnp.arange(B) * S).reshape(B, 1)
        flat_idx = (idx + b_off).reshape(B * C)
        zero = (x * 0.0).reshape(B * S, D)
        upd = _scatter_add(zero, flat_idx, y.reshape(B * C, D), axis=0)
        return x + upd.reshape(B, S, D)

    x = A_x
    xn = _layernorm(x, axis=-1)
    s = _A_ref(xn, A_wqkv, A_wo)
    g = _silu(_B_ref(xn, B_w_r, B_w_gate, B_w_up, B_w_down))
    return x + s * g
```

```python
import numpy as np
import jax
import jax.numpy as jnp
from jax import lax
import jax.experimental.pallas as pl
import jax.experimental.pallas.tpu as pltpu

S, D, H, W, DIL, F = 2048, 640, 32, 8, 2, 1728
DH = D // H
NJ = D // 128
T = 256
NB = S // T
HALO = 16
RC = 16
UNROLL = 0
F32, BF16 = jnp.float32, jnp.bfloat16
EPS = 1.00135803e-05
SCALE = DH ** -0.5
NEG = -999292928.0
LOG2E = 1.4426950408889634
NT = (((1,), (1,)), ((), ()))


def _rb(x):
    return x.astype(BF16).astype(F32)


def kernel(x_hbm, wqkv_hbm, wo_hbm, wr_ref, wg_hbm, wu_hbm, wd_hbm, out_hbm,
           x_v, xn_v, o_v, out_v, wqkv_v, wt_v, wo_v, wop_v, wg_v, wu_v, wd_v, tmp_v,
           xa_v, xb_v, qa_v, qb_v, ka_v, kb_v, va_v, vb_v, r_v,
           sem_x, sem_w, sem_o):
    def x_copy(i):
        return pltpu.make_async_copy(x_hbm.at[pl.ds(i * T, T)], x_v.at[pl.ds(i * T, T)], sem_x.at[i])

    def wqkv_copy(p):
        return pltpu.make_async_copy(wqkv_hbm.at[:, pl.ds(p * D, D)], wqkv_v.at[p], sem_w.at[p])

    wo_copy = pltpu.make_async_copy(wo_hbm, wo_v, sem_w.at[3])
    wg_copy = pltpu.make_async_copy(wg_hbm, wg_v, sem_w.at[4])
    wu_copy = pltpu.make_async_copy(wu_hbm, wu_v, sem_w.at[5])
    wd_copy = pltpu.make_async_copy(wd_hbm, wd_v, sem_w.at[6])

    def out_copy(i):
        return pltpu.make_async_copy(out_v.at[pl.ds(i * T, T)], out_hbm.at[pl.ds(i * T, T)], sem_o.at[i])

    wqkv_copy(0).start()
    x_copy(0).start()
    wqkv_copy(1).start()
    wqkv_copy(2).start()
    for i in range(1, NB):
        x_copy(i).start()
    wo_copy.start()
    wg_copy.start()
    wu_copy.start()
    wd_copy.start()

    def prep_wqkv(p):
        for kt in range(NJ):
            tmp_v[kt] = wqkv_v[p, pl.ds(kt * 128, 128), :].astype(F32).T
        for kt in range(NJ):
            for d in range(DH):
                wt_v[p, pl.ds(d * H, H), pl.ds(kt * 128, 128)] = tmp_v[kt, pl.ds(d, H, stride=DH), :].astype(BF16)

    def prep_wo():
        for j in range(NJ):
            tmp_v[j] = wo_v[:, pl.ds(j * 128, 128)].astype(F32)
        for j in range(NJ):
            for d in range(DH):
                wop_v[pl.ds(d * H, H), pl.ds(j * 128, 128)] = tmp_v[j, pl.ds(d, H, stride=DH), :].astype(BF16)

    def rows(i, r0, n):
        if isinstance(i, int):
            return pl.ds(i * T + r0, n)
        return pl.ds(pl.multiple_of(i * T + r0, 16), n)

    def ln(i, xdst):
        wr = wr_ref[...].astype(F32).reshape(1, D)
        lane = lax.broadcasted_iota(jnp.int32, (RC, 128), 1)
        racc = jnp.zeros((RC, 128), F32)
        for c in range(T // RC):
            xf = x_v[rows(i, c * RC, RC), :].astype(F32)
            mean = jnp.sum(xf, axis=-1, keepdims=True) * (1.0 / D)
            cen = xf - mean
            var = jnp.sum(cen * cen, axis=-1, keepdims=True) * (1.0 / D)
            sd = _rb(jnp.sqrt(_rb(_rb(var) + EPS)))
            xn = (_rb(xf - _rb(mean)) * (1.0 / sd)).astype(BF16)
            xdst[pl.ds(c * RC, RC), :] = xn
            xn_v[rows(i, c * RC, RC), :] = xn
            r = jnp.sum(xn.astype(F32) * wr, axis=-1, keepdims=True)
            racc = jnp.where(lane == c, r, racc)
        r_v[i] = racc

    def qkv_part(p, xsrc, dst, off):
        res = lax.dot_general(xsrc[...], wt_v[p], NT, preferred_element_type=F32)
        for j in range(NJ):
            dst[j, pl.ds(off, T), :] = res[:, j * 128:(j + 1) * 128]

    def qkv(xsrc, q, k, v):
        qkv_part(0, xsrc, q, 0)
        qkv_part(1, xsrc, k, HALO)
        qkv_part(2, xsrc, v, HALO)

    def halo(ksrc, vsrc, kdst, vdst):
        kdst[:, pl.ds(0, HALO), :] = ksrc[:, pl.ds(T, HALO), :]
        vdst[:, pl.ds(0, HALO), :] = vsrc[:, pl.ds(T, HALO), :]

    def attn(i, q, k, v, first=False):
        for c in range(T // RC):
            r0 = c * RC
            qs = [q[j, pl.ds(r0, RC), :] for j in range(NJ)]
            ls = []
            for w in range(W):
                a = None
                for j in range(NJ):
                    t = qs[j] * k[j, pl.ds(HALO + r0 - DIL * w, RC), :]
                    a = t if a is None else a + t
                a = a + pltpu.roll(a, 64, 1)
                a = a + pltpu.roll(a, 32, 1)
                if first and r0 < DIL * w:
                    pos = lax.broadcasted_iota(jnp.int32, (RC, 128), 0) + r0
                    a = jnp.where(pos >= DIL * w, a, NEG / SCALE)
                ls.append(a)
            m = ls[0]
            for w in range(1, W):
                m = jnp.maximum(m, ls[w])
            es = [jnp.exp2((l - m) * (SCALE * LOG2E)) for l in ls]
            den = es[0]
            for w in range(1, W):
                den = den + es[w]
            inv = 1.0 / den
            for j in range(NJ):
                acc = None
                for w in range(W):
                    t = es[w] * v[j, pl.ds(HALO + r0 - DIL * w, RC), :]
                    acc = t if acc is None else acc + t
                o_v[rows(i, r0, RC), pl.ds(j * 128, 128)] = (acc * inv).astype(BF16)

    def route_and_ffn():
        r = _rb(r_v[...].reshape(NB * RC, 128)) + 0.0
        row = lax.broadcasted_iota(jnp.int32, (NB * RC, 128), 0)
        lane = lax.broadcasted_iota(jnp.int32, (NB * RC, 128), 1)
        tok = (row // RC) * T + lane * RC + row % RC
        bits = lax.bitcast_convert_type(r, jnp.int32)
        key = jnp.where(bits >= 0, bits, bits ^ 0x7FFFFFFF)
        imin = -2 ** 31
        key = jnp.where(r != r, imin + 1, key)
        key = jnp.where(lane < T // RC, key, imin)
        sel = []
        for _ in range(2):
            kmax = jnp.max(key)
            idx = jnp.min(jnp.where(key == kmax, tok, S))
            rsel = jnp.sum(jnp.where(tok == idx, jnp.where(lane < T // RC, r, 0.0), 0.0))
            key = jnp.where(tok == idx, imin, key)
            sel.append((idx, rsel))
        bases = [pl.multiple_of(jnp.clip((idx // 16) * 16, 0, S - 16), 16) for idx, _ in sel]
        xs = jnp.concatenate([xn_v[pl.ds(b, 16), :] for b in bases], axis=0)
        g = _rb(lax.dot_general(xs, wg_v[...], NT, preferred_element_type=F32))
        u = _rb(lax.dot_general(xs, wu_v[...], NT, preferred_element_type=F32))
        hdn = (_rb(g * jax.nn.sigmoid(g)) * u).astype(BF16)
        y = _rb(jnp.dot(hdn, wd_v[...], preferred_element_type=F32))
        rr = lax.broadcasted_iota(jnp.int32, (16, D), 0)
        for n, ((idx, rsel), b) in enumerate(zip(sel, bases)):
            gate = _rb(jax.nn.sigmoid(jnp.full((16, D), rsel, F32)))
            upd = jnp.where(rr == idx - b, _rb(y[n * 16:(n + 1) * 16] * gate), 0.0)
            xn_v[pl.ds(b, 16), :] = (xn_v[pl.ds(b, 16), :].astype(F32) + upd).astype(BF16)

    def outproj(i):
        s = jnp.dot(o_v[rows(i, 0, T), :], wop_v[...], preferred_element_type=F32)
        for c in range(T // RC):
            z = xn_v[rows(i, c * RC, RC), :].astype(F32)
            xf = x_v[rows(i, c * RC, RC), :].astype(F32)
            out_v[rows(i, c * RC, RC), :] = (xf + s[c * RC:(c + 1) * RC] * (z * jax.nn.sigmoid(z))).astype(BF16)

    A = (xa_v, qa_v, ka_v, va_v)
    B = (xb_v, qb_v, kb_v, vb_v)

    x_copy(0).wait()
    ln(0, xa_v)
    wqkv_copy(0).wait()
    prep_wqkv(0)
    qkv_part(0, xa_v, qa_v, 0)
    wqkv_copy(1).wait()
    prep_wqkv(1)
    qkv_part(1, xa_v, ka_v, HALO)
    wqkv_copy(2).wait()
    prep_wqkv(2)
    qkv_part(2, xa_v, va_v, HALO)
    ka_v[:, pl.ds(0, HALO), :] = jnp.broadcast_to(ka_v[:, pl.ds(HALO, 1), :], (NJ, HALO, 128))
    va_v[:, pl.ds(0, HALO), :] = jnp.broadcast_to(va_v[:, pl.ds(HALO, 1), :], (NJ, HALO, 128))
    for i in range(1, NB):
        x_copy(i).wait()
    ln(1, xb_v)

    def step(i, cur, prev, first=False, do_ln=True):
        halo(prev[2], prev[3], cur[2], cur[3])
        qkv(*cur)
        attn(i - 1, prev[1], prev[2], prev[3], first=first)
        if do_ln:
            ln(i + 1, prev[0])

    step(1, B, A, first=True)
    if UNROLL:
        for i in range(2, NB - 1):
            step(i, A if i % 2 == 0 else B, B if i % 2 == 0 else A)
    else:
        def body(n, carry):
            step(2 * n, A, B)
            step(2 * n + 1, B, A)
            return carry
        lax.fori_loop(1, NB // 2 - 1, body, 0)
        step(NB - 2, A, B)
    step(NB - 1, B, A, do_ln=False)
    wo_copy.wait()
    prep_wo()
    wg_copy.wait()
    wu_copy.wait()
    wd_copy.wait()
    route_and_ffn()
    attn(NB - 1, qb_v, kb_v, vb_v)
    if UNROLL:
        for i in range(NB):
            outproj(i)
            out_copy(i).start()
    else:
        def body2(i, carry):
            outproj(i)
            out_copy(i).start()
            return carry
        lax.fori_loop(0, NB, body2, 0)
    for i in range(NB):
        out_copy(i).wait()


@jax.jit
def pallas_recurrent_scan__sliding_local_dilated__moe_arch_mod__prompt_kernel(
    A_x, A_wqkv, A_wo, B_x, B_w_r, B_w_gate, B_w_up, B_w_down,
):
    any_spec = pl.BlockSpec(memory_space=pltpu.HBM)
    V = pltpu.VMEM
    out = pl.pallas_call(
        kernel,
        out_shape=jax.ShapeDtypeStruct((S, D), BF16),
        in_specs=[any_spec, any_spec, any_spec, pl.BlockSpec(memory_space=pltpu.VMEM), any_spec, any_spec, any_spec],
        out_specs=any_spec,
        scratch_shapes=[
            V((S, D), BF16), V((S, D), BF16), V((S, D), BF16), V((S, D), BF16),
            V((3, D, D), BF16), V((3, D, D), BF16), V((D, D), BF16), V((D, D), BF16),
            V((F, D), BF16), V((F, D), BF16), V((F, D), BF16), V((NJ, D, 128), F32),
            V((T, D), BF16), V((T, D), BF16),
            V((NJ, T, 128), F32), V((NJ, T, 128), F32),
            V((NJ, T + HALO, 128), F32), V((NJ, T + HALO, 128), F32),
            V((NJ, T + HALO, 128), F32), V((NJ, T + HALO, 128), F32),
            V((NB, RC, 128), F32),
            pltpu.SemaphoreType.DMA((NB,)), pltpu.SemaphoreType.DMA((7,)), pltpu.SemaphoreType.DMA((NB,)),
        ],
        compiler_params=pltpu.CompilerParams(vmem_limit_bytes=100 * 1024 * 1024),
    )(A_x.reshape(S, D), A_wqkv, A_wo, B_w_r, B_w_gate.T, B_w_up.T, B_w_down)
    return out.reshape(1, S, D)
```

```python
import jax
import jax.numpy as jnp
from jax import lax
import jax.experimental.pallas as pl
import jax.experimental.pallas.tpu as pltpu

S, D, H, W, DIL, F = 2048, 640, 32, 8, 2, 1728
DH = D // H
NJ = D // 128
T = 256
NB = S // T
HALO = 16
RC = 16
AR = 8
NF = pl.cdiv(F, 128)
GA = 3
GL = 1
SPAN = 90
BAR = 1
FFN0 = 3
LNP = 48
SCOPES = 0
LP = 0
F32, BF16 = jnp.float32, jnp.bfloat16
EPS = 1.00135803e-05
SCALE = DH ** -0.5
NEG = -999292928.0
LOG2E = 1.4426950408889634
NT = (((1,), (1,)), ((), ()))


def _rb(x):
    return x.astype(BF16).astype(F32)


def _silu(z):
    h = 0.5 * z
    return h + h * jnp.tanh(h)


def _sum(t):
    a = t[0]
    for b in t[1:]:
        a = a + b
    return a


def _tiles(x):
    return [x[:, j * 128:(j + 1) * 128] for j in range(NJ)]


def _row(ref, r0, n):
    return jnp.concatenate([ref[j, pl.ds(r0, n), :] for j in range(NJ)], axis=1)


class _NoScope:
    def __enter__(self):
        return self

    def __exit__(self, *a):
        return False


def scope(name):
    return jax.named_scope(name) if SCOPES else _NoScope()


def kernel(x_hbm, wqkv_hbm, wo_hbm, wr_hbm, wg_hbm, wu_hbm, wd_hbm, out_hbm,
           x_v, xn_v, q_v, k_v, v_v, o_v, out_v, wr_v, wqkv_v, wt_v, wo_v, wop_v, wg_v, wu_v, wd_v, tmp_v,
           r_v, xs_v, h_v, y_v, idx_s, sem_x, sem_w, sem_f, sem_o):
    XB = [(0, T), (T, 2 * T), (3 * T, S - 3 * T)]
    OB = [(0, 3 * T), (3 * T, 3 * T), (6 * T, T + T // 2), (7 * T + T // 2, T // 2)]

    def x_copy(n):
        r0, nr = XB[n]
        return pltpu.make_async_copy(x_hbm.at[pl.ds(r0, nr)], x_v.at[pl.ds(r0, nr)], sem_x.at[n])

    def wqkv_copy(p):
        return pltpu.make_async_copy(wqkv_hbm.at[:, pl.ds(p * D, D)], wqkv_v.at[p], sem_w.at[p])

    def wo_copy():
        return pltpu.make_async_copy(wo_hbm, wo_v, sem_w.at[3])

    def wr_copy():
        return pltpu.make_async_copy(wr_hbm, wr_v, sem_w.at[4])

    def ffn_copies():
        return [pltpu.make_async_copy(src.at[:, pl.ds(j * 128, 128)], dst.at[j], sem_f.at[m, j])
                for m, (src, dst) in enumerate(((wg_hbm, wg_v), (wu_hbm, wu_v), (wd_hbm, wd_v))) for j in range(NJ)]

    def out_copy(n):
        r0, nr = OB[n]
        return pltpu.make_async_copy(out_v.at[pl.ds(r0, nr)], out_hbm.at[pl.ds(r0, nr)], sem_o.at[n])

    def prep_wqkv(p):
        for kt in range(NJ):
            tmp_v[kt] = wqkv_v[p, pl.ds(kt * 128, 128), :].astype(F32).T
        for kt in range(NJ):
            for d in range(DH):
                wt_v[p, kt, pl.ds(d * H, H), :] = tmp_v[kt, pl.ds(d, H, stride=DH), :].astype(BF16)

    def prep_wo():
        for j in range(NJ):
            tmp_v[j] = wo_v[:, pl.ds(j * 128, 128)].astype(F32)
        for j in range(NJ):
            for d in range(DH):
                wop_v[j, pl.ds(d * H, H), :] = tmp_v[j, pl.ds(d, H, stride=DH), :].astype(BF16)

    def always(n):
        bits = lax.bitcast_convert_type(wr_v[...].astype(F32).reshape(1, D)[:, :128], jnp.int32)
        return jnp.broadcast_to(bits | 1, (n, 128)) != 0

    def pacer(res):
        keep = {n: always(n) for n in (AR, RC)}

        def pace(x, frac):
            if frac < 0:
                return x
            n = x.shape[0]
            pos = min(frac * SPAN / 100, 0.98) * len(res)
            tile = int(pos)
            m = res[tile].shape[0]
            r0 = min(int((pos - tile) * m) // 8 * 8, m - n)
            return jnp.where(keep[n], x, res[tile][r0:r0 + n])
        return pace

    def no_pace(x, frac):
        return x

    def ln(c0, c1, pace=no_pace):
        wr = wr_v[...].astype(F32).reshape(1, D)
        lane = lax.broadcasted_iota(jnp.int32, (RC, 128), 1)
        racc = r_v[...]
        for c in range(c0, c1):
            xf = x_v[pl.ds(c * RC, RC), :].astype(F32)
            part = pace(_sum(_tiles(xf)), (c - c0 - GL) / (c1 - c0))
            mean = jnp.sum(part, axis=-1, keepdims=True) * (1.0 / D)
            mb = _rb(mean)
            xc = xf - mb
            dm = mean - mb
            var = jnp.maximum(jnp.sum(xc * xc, axis=-1, keepdims=True) * (1.0 / D) - dm * dm, 0.0)
            sd = _rb(jnp.sqrt(_rb(_rb(var) + EPS)))
            xn = _rb(_rb(xc) * (1.0 / sd))
            for j, t in enumerate(_tiles(xn)):
                xn_v[j, pl.ds(c * RC, RC), :] = t
            racc = jnp.where(lane == c, jnp.sum(xn * wr, axis=-1, keepdims=True), racc)
        r_v[...] = racc

    def qkv_tile(i, p, j):
        dst, off = [(q_v, 0), (k_v, HALO), (v_v, HALO)][p]
        res = lax.dot_general(_row(xn_v, i * T, T), _row(wt_v.at[p], j * 128, 128), NT, preferred_element_type=F32)
        dst[j, pl.ds(off + i * T, T), :] = res
        return res

    def qkv_part(i, p):
        dst, off = [(q_v, 0), (k_v, HALO), (v_v, HALO)][p]
        rhs = jnp.concatenate([wt_v[p, kt] for kt in range(NJ)], axis=1)
        res = _tiles(lax.dot_general(_row(xn_v, i * T, T), rhs, NT, preferred_element_type=F32))
        for j, t in enumerate(res):
            dst[j, pl.ds(off + i * T, T), :] = t
        return res

    def attn(i, pace=no_pace):
        nc = T // AR
        for c in range(nc):
            r0 = i * T + c * AR
            qs = [q_v[j, pl.ds(r0, AR), :] for j in range(NJ)]
            ls = []
            for w in range(W):
                a = _sum([qs[j] * k_v[j, pl.ds(HALO + r0 - DIL * w, AR), :] for j in range(NJ)])
                ls.append(pace(a, (c - GA + w / W) / nc))
            ls = [a + pltpu.roll(a, 64, 1) for a in ls]
            ls = [a + pltpu.roll(a, 32, 1) for a in ls]
            for w in range(W):
                if r0 < DIL * w:
                    pos = lax.broadcasted_iota(jnp.int32, (AR, 128), 0) + r0
                    ls[w] = jnp.where(pos >= DIL * w, ls[w], NEG / SCALE)
            mx = jnp.maximum
            m = mx(mx(mx(ls[0], ls[1]), mx(ls[2], ls[3])), mx(mx(ls[4], ls[5]), mx(ls[6], ls[7])))
            es = [jnp.exp2((l - m) * (SCALE * LOG2E)) for l in ls]
            den = _sum(es)
            inv = pltpu.reciprocal(den, approx=True)
            inv = inv * (2.0 - den * inv)
            for j in range(NJ):
                o_v[j, pl.ds(r0, AR), :] = inv * _sum(
                    [es[w] * v_v[j, pl.ds(HALO + r0 - DIL * w, AR), :] for w in range(W)])

    def route():
        r = _rb(r_v[...]) + 0.0
        tok = (lax.broadcasted_iota(jnp.int32, (RC, 128), 1) * RC
               + lax.broadcasted_iota(jnp.int32, (RC, 128), 0))
        bits = lax.bitcast_convert_type(r, jnp.int32)
        imin = -2 ** 31
        key = jnp.where(bits >= 0, bits, bits ^ 0x7FFFFFFF)
        key = jnp.where(r != r, imin + 1, key)
        sub = lax.broadcasted_iota(jnp.int32, (8, D), 0)
        xs = jnp.zeros((8, D), F32)
        gate = jnp.zeros((8, D), F32)
        for n in range(2):
            kmax = jnp.max(key, keepdims=True)
            hit = jnp.min(jnp.where(key == kmax, tok, S - 1), keepdims=True)
            rsel = jnp.sum(jnp.where(tok == hit, r, 0.0), keepdims=True)
            key = jnp.where(tok == hit, imin, key)
            idx = jnp.clip(hit[0, 0], 0, S - 1)
            idx_s[n] = idx
            xs = jnp.where(sub == n, _row(xn_v, idx, 1), xs)
            gate = jnp.where(sub == n, rsel, gate)
        xs_v[0] = xs
        xs_v[1] = _rb(jax.nn.sigmoid(gate))
        y_v[...] = jnp.zeros_like(y_v)

    def ffn_ops():
        def gate(n, r0, nr):
            g = _rb(lax.dot_general(xs_v[0], _row(wg_v, r0, nr), NT, preferred_element_type=F32))
            h_v[n, :, pl.ds(0, nr)] = _rb(_silu(g))

        def up(n, r0, nr):
            u = _rb(lax.dot_general(xs_v[0], _row(wu_v, r0, nr), NT, preferred_element_type=F32))
            h_v[n, :, pl.ds(0, nr)] = _rb(h_v[n, :, pl.ds(0, nr)] * u)

        def down(n, r0, nr):
            y_v[...] += jnp.dot(h_v[n, :, pl.ds(0, nr)], _row(wd_v, r0, nr), preferred_element_type=F32)
        return [lambda f=f, n=n: f(n, n * 128, min(128, F - n * 128)) for f in (gate, up, down) for n in range(NF)]

    def scatter():
        y = _rb(_rb(y_v[...]) * xs_v[1])
        for n in range(2):
            idx = jnp.clip(idx_s[n], 0, S - 1)
            for j, t in enumerate(_tiles(y[n:n + 1])):
                xn_v[j, pl.ds(idx, 1), :] = _rb(xn_v[j, pl.ds(idx, 1), :] + t)

    def outproj(r0, nr):
        rhs = jnp.concatenate([wop_v[j] for j in range(NJ)], axis=1)
        s = jnp.dot(_row(o_v, r0, nr), rhs, preferred_element_type=F32)
        for c in range(0, nr, RC):
            xf = x_v[pl.ds(r0 + c, RC), :].astype(F32)
            out_v[pl.ds(r0 + c, RC), :] = (xf + s[c:c + RC] * _silu(_row(xn_v, r0 + c, RC))).astype(BF16)
        return _tiles(s)

    with scope("z0_pro"):
        x_copy(0).start()
        wr_copy().start()
        wqkv_copy(0).start()
        r_v[...] = jnp.zeros_like(r_v)
        x_copy(0).wait()
        wr_copy().wait()
        wqkv_copy(1).start()
        ln(0, T // RC)
        wqkv_copy(0).wait()
        wqkv_copy(2).start()
        prep_wqkv(0)
        wqkv_copy(1).wait()
        x_copy(1).start()
        qkv_part(0, 0)
        prep_wqkv(1)
        wqkv_copy(2).wait()
        x_copy(2).start()
        qkv_part(0, 1)
        prep_wqkv(2)
        x_copy(1).wait()
        res = qkv_part(0, 2)
        ln(T // RC, LNP, pacer(res))
        for buf in (k_v, v_v):
            buf[:, pl.ds(0, HALO), :] = jnp.broadcast_to(buf[:, pl.ds(HALO, 1), :], (NJ, HALO, 128))
        x_copy(2).wait()
        wo_copy().start()
        for c in ffn_copies():
            c.start()

    def block(f):
        if BAR:
            pl.when(idx_s[2] == 1)(f)
        else:
            f()

    if BAR:
        idx_s[2] = (jnp.max(lax.bitcast_convert_type(r_v[...], jnp.int32)) | 1) & 1

    NL = NB - 4
    with scope("z8_loop"):
        for i in range(1, NL + 1):
            def step(i=i):
                pace = pacer([t for p in range(3) for t in qkv_part(i, p)])
                attn(i - 1, pace)
                left = S // RC - LNP
                ln(LNP + left * (i - 1) // NL, LNP + left * i // NL, pace)
            block(step)
    with scope("z9_ffn"):
        wo_copy().wait()
        for c in ffn_copies():
            c.wait()
        ffn = [None] * FFN0 + ffn_ops()
        for i in range(NL + 1, NB):
            def step(i=i):
                if i == NL + 1:
                    route()
                res = []
                for p in range(3):
                    for j in range(NJ):
                        res.append(qkv_tile(i, p, j))
                        op = ffn.pop(0) if ffn else None
                        if op is not None:
                            op()
                attn(i - 1, pacer(res))
                if i == NB - 2:
                    prep_wo()
                if i == NB - 1:
                    for op in ffn:
                        op()
                    scatter()
            block(step)
    with scope("zb_out"):
        for n, (r0, nr) in enumerate(OB):
            res = [t for b0 in range(r0, r0 + nr, T) for t in outproj(b0, min(T, r0 + nr - b0))]
            if n == 0:
                attn(NB - 1, pacer(res))
            out_copy(n).start()
        for n in range(len(OB)):
            out_copy(n).wait()


@jax.jit
def pallas_recurrent_scan__sliding_local_dilated__moe_arch_mod__prompt_kernel(
    A_x, A_wqkv, A_wo, B_x, B_w_r, B_w_gate, B_w_up, B_w_down,
):
    hbm = pl.BlockSpec(memory_space=pltpu.HBM)
    V = pltpu.VMEM
    dma = pltpu.SemaphoreType.DMA
    flags = {"XLA_TPU_EVENLY_DISTRIBUTE_CRITICAL_NODES": True} if LP else None
    out = pl.pallas_call(
        kernel,
        out_shape=jax.ShapeDtypeStruct((S, D), BF16),
        in_specs=[hbm] * 7,
        out_specs=hbm,
        scratch_shapes=[
            V((S, D), BF16), V((NJ, S, 128), F32),
            V((NJ, S, 128), F32), V((NJ, S + HALO, 128), F32), V((NJ, S + HALO, 128), F32),
            V((NJ, S, 128), F32), V((S, D), BF16),
            V((D,), BF16), V((3, D, D), BF16), V((3, NJ, D, 128), BF16), V((D, D), BF16), V((NJ, D, 128), BF16),
            V((NJ, F, 128), BF16), V((NJ, F, 128), BF16), V((NJ, F, 128), BF16), V((NJ, D, 128), F32),
            V((RC, 128), F32), V((2, 8, D), F32), V((NF, 8, 128), F32), V((8, D), F32),
            pltpu.SMEM((3,), jnp.int32),
            dma((3,)), dma((5,)), dma((3, NJ)), dma((4,)),
        ],
        compiler_params=pltpu.CompilerParams(vmem_limit_bytes=100 * 1024 * 1024, flags=flags),
    )(A_x.reshape(S, D), A_wqkv, A_wo, B_w_r, B_w_gate.T, B_w_up.T, B_w_down)
    return out.reshape(1, S, D)
```

```python
import jax
import jax.numpy as jnp
from jax import lax
import jax.experimental.pallas as pl
import jax.experimental.pallas.tpu as pltpu

S, D, H, W, DIL, F = 2048, 640, 32, 8, 2, 1728
DH = D // H
NJ = D // 128
T = 256
HALO = 16
RC = 16
AR = 8
NF = pl.cdiv(F, 128)
GA = 15
GL = 15
G2 = 5
PLAN = 0
ONLY = -1
SCOPES = 0
LP = 0
F32, BF16, U32 = jnp.float32, jnp.bfloat16, jnp.uint32
EPS = 1.00135803e-05
SCALE = DH ** -0.5
NEG = -999292928.0
LOG2E = 1.4426950408889634
NT = (((1,), (1,)), ((), ()))
Q, K, V = 0, 1, 2
FIRST, LAST = range(NJ - 1), [NJ - 1]
X_BLOCKS = [(0, T), (T, T), (2 * T, T), (3 * T, S - 3 * T)]
OUT_BLOCKS = [(i * T, T) for i in range(7)] + [(7 * T, 128), (7 * T + 128, 64), (7 * T + 192, 64)]
PLANS = {
    0: ([(0, V, 0, 10), (1, V, 6, 8), (2, Q, 8, 8), (2, K, 8, 8), (2, V, 6, 6)],
        [(3, Q, 8, 9), (3, K, 8, 9), (3, V, 8, 9), (4, Q, 8, 9), (4, K, 9, 4), (4, V, 9, 0)],
        [13, 13, 13, 11, 11, 11, 13, 13, 12],
        [12, 12, 12, 12, 10, 10, 0, 0, 0, 0]),
    1: ([(0, V, 0, 10), (1, V, 7, 8), (2, Q, 9, 8), (2, K, 9, 8), (2, V, 7, 6)],
        [(3, Q, 9, 9), (3, K, 9, 9), (3, V, 9, 9), (4, Q, 9, 9), (4, K, 10, 4), (4, V, 10, 0)],
        [12, 12, 12, 10, 10, 10, 12, 12, 11],
        [12, 12, 12, 12, 12, 7, 0, 0, 0, 0]),
    2: ([(0, V, 0, 12), (1, V, 7, 8), (2, Q, 8, 8), (2, K, 8, 8), (2, V, 7, 6)],
        [(3, Q, 8, 9), (3, K, 8, 9), (3, V, 8, 9), (4, Q, 9, 8), (4, K, 11, 3), (4, V, 10, 0)],
        [12, 12, 12, 10, 10, 10, 12, 12, 10],
        [13, 13, 13, 13, 12, 8, 0, 0, 0, 0]),
}


def _rb(x):
    return x.astype(BF16).astype(F32)


def _silu(z):
    h = 0.5 * z
    return h + h * jnp.tanh(h)


def _sum(t):
    a = t[0]
    for b in t[1:]:
        a = a + b
    return a


def _tiles(x):
    return [x[:, j * 128:(j + 1) * 128] for j in range(x.shape[1] // 128)]


def _words(x):
    return pltpu.bitcast(x.astype(BF16), U32)


def _row(ref, r0, n, js=range(NJ)):
    if ref.dtype == U32:
        return jnp.concatenate([pltpu.bitcast(ref[j, pl.ds(r0 // 2, n // 2), :], BF16) for j in js], axis=1)
    return jnp.concatenate([ref[j, pl.ds(r0, n), :] for j in js], axis=1)


def _nt(a, b):
    return lax.dot_general(a, b, NT, preferred_element_type=F32)


class _NoScope:
    def __enter__(self):
        return self

    def __exit__(self, *a):
        return False


def scope(name):
    return jax.named_scope(name) if SCOPES else _NoScope()


def kernel(x_hbm, wqkv_hbm, wo_hbm, wr_hbm, wg_hbm, wu_hbm, wd_hbm, out_hbm,
           x_v, xn_v, q_v, k_v, v_v, o_v, out_v, wr_v, wqkv_v, wt_v, wo_v, wop_v, wg_v, wu_v, wd_v, tmp_v,
           r_v, xs_v, y_v, idx_s, sem_x, sem_w, sem_f, sem_o):
    def x_copy(n):
        r0, nr = X_BLOCKS[n]
        return pltpu.make_async_copy(x_hbm.at[pl.ds(r0, nr)], x_v.at[pl.ds(r0, nr)], sem_x.at[n])

    def wq_copy(kt):
        rows = pl.ds(kt * 128, 128)
        return pltpu.make_async_copy(wqkv_hbm.at[rows, pl.ds(0, D)], wqkv_v.at[Q, rows], sem_w.at[kt])

    def wkv_copy(p):
        return pltpu.make_async_copy(wqkv_hbm.at[:, pl.ds(p * D, D)], wqkv_v.at[p], sem_w.at[NJ - 1 + p])

    def wo_copy():
        return pltpu.make_async_copy(wo_hbm, wo_v, sem_w.at[NJ + 2])

    def wr_copy():
        return pltpu.make_async_copy(wr_hbm, wr_v, sem_w.at[NJ + 3])

    def ffn_copies():
        return [pltpu.make_async_copy(src.at[:, pl.ds(j * 128, 128)], dst.at[j], sem_f.at[m, j])
                for m, (src, dst) in enumerate(((wg_hbm, wg_v), (wu_hbm, wu_v), (wd_hbm, wd_v))) for j in range(NJ)]

    def out_copy(n):
        r0, nr = OUT_BLOCKS[n]
        return pltpu.make_async_copy(out_v.at[pl.ds(r0, nr)], out_hbm.at[pl.ds(r0, nr)], sem_o.at[n])

    class Pacer:
        def __init__(self):
            self.tiles = []
            bits = lax.bitcast_convert_type(wr_v[...].astype(F32).reshape(1, D)[:, :128], jnp.int32)
            self.keep = jnp.broadcast_to(bits | 1, (AR, 128)) != 0

        def add(self, tiles):
            self.start = len(self.tiles)
            self.tiles += tiles

        def __call__(self, x, frac, lead):
            pos = self.start + frac * (len(self.tiles) - self.start) - lead / 10
            if pos < 0:
                return x
            tile = self.tiles[min(int(pos), len(self.tiles) - 1)]
            r0 = int(pos % 1 * tile.shape[0]) // AR * AR
            return jnp.concatenate([jnp.where(self.keep, x[r:r + AR], tile[r0:r0 + AR])
                                    for r in range(0, x.shape[0], AR)], axis=0)

    def no_pace(x, frac, lead):
        return x

    def prep_wqkv(p, kts=range(NJ), pace=no_pace):
        for kt in kts:
            tmp_v[kt] = wqkv_v[p, pl.ds(kt * 128, 128), :].astype(F32).T
        for kt in kts:
            for d in range(DH):
                wt_v[kt, pl.ds((p * D + d * H) // 2, H // 2), :] = _words(tmp_v[kt, pl.ds(d, H, stride=DH), :])

    def prep_wo(j, pace):
        for r in range(0, D, 64):
            tmp_v[j, pl.ds(r, 64), :] = pace(wo_v[pl.ds(r, 64), pl.ds(j * 128, 128)].astype(F32), r / D / 2, 0)
        for d in range(DH):
            wop_v[j, pl.ds(d * H // 2, H // 2), :] = _words(tmp_v[j, pl.ds(d, H, stride=DH), :])

    def ln(c0, n, pace=no_pace):
        if n == 0:
            return
        wr = wr_v[...].astype(F32).reshape(1, D)
        lane = lax.broadcasted_iota(jnp.int32, (RC, 128), 1)
        racc = r_v[...]
        for c in range(c0, c0 + n):
            xf = x_v[pl.ds(c * RC, RC), :].astype(F32)
            part = pace(_sum(_tiles(xf)), (c - c0) / n, GL)
            mean = jnp.sum(part, axis=-1, keepdims=True) * (1.0 / D)
            mb = _rb(mean)
            xc = xf - mb
            dm = mean - mb
            part = _sum(_tiles(xc * xc))
            if G2:
                part = pace(part, (c - c0) / n, GL - G2)
            var = jnp.maximum(jnp.sum(part, axis=-1, keepdims=True) * (1.0 / D) - dm * dm, 0.0)
            sd = _rb(jnp.sqrt(_rb(_rb(var) + EPS)))
            xn = _rb(_rb(xc) * pltpu.reciprocal(sd, full_range=False))
            for j, t in enumerate(_tiles(xn)):
                xn_v[j, pl.ds(c * RC, RC), :] = t
            racc = jnp.where(lane == c, jnp.sum(xn * wr, axis=-1, keepdims=True), racc)
        r_v[...] = racc

    def qkv_tile(i, n):
        dst, off = [(q_v, 0), (k_v, HALO), (v_v, HALO)][n // NJ]
        return dst.at[n % NJ, pl.ds(off + i * T, T)]

    def proj(i, p):
        res = _tiles(_nt(_row(xn_v, i * T, T), _row(wt_v, p * D, D)))
        for j, t in enumerate(res):
            qkv_tile(i, p * NJ + j)[...] = t
            if i == 0 and p != Q:
                (k_v, v_v)[p - K][j, pl.ds(0, HALO), :] = jnp.broadcast_to(t[0:1], (HALO, 128))
        return res

    def proj_pieces(i):
        for n0 in range(0, 3 * NJ, 4):
            ns = range(n0, min(n0 + 4, 3 * NJ))
            part = _nt(_row(xn_v, i * T, T, LAST), _row(wt_v, n0 * 128, len(ns) * 128, LAST))
            yield []
            for n, t in zip(ns, _tiles(part)):
                res = t + _nt(_row(xn_v, i * T, T, FIRST), _row(wt_v, n * 128, 128, FIRST))
                qkv_tile(i, n)[...] = res
                yield [res]

    def attn(c0, n, pace):
        for c in range(c0, c0 + n):
            r0 = c * AR
            qs = [q_v[j, pl.ds(r0, AR), :] for j in range(NJ)]
            ls = []
            for w in range(W):
                a = _sum([qs[j] * k_v[j, pl.ds(HALO + r0 - DIL * w, AR), :] for j in range(NJ)])
                ls.append(pace(a, (c - c0 + w / W) / n, GA))
            ls = [a + pltpu.roll(a, 64, 1) for a in ls]
            ls = [a + pltpu.roll(a, 32, 1) for a in ls]
            for w in range(W):
                if r0 < DIL * w:
                    pos = lax.broadcasted_iota(jnp.int32, (AR, 128), 0) + r0
                    ls[w] = jnp.where(pos >= DIL * w, ls[w], NEG / SCALE)
            mx = jnp.maximum
            m = mx(mx(mx(ls[0], ls[1]), mx(ls[2], ls[3])), mx(mx(ls[4], ls[5]), mx(ls[6], ls[7])))
            es = [jnp.exp2((l - m) * (SCALE * LOG2E)) for l in ls]
            den = _sum(es)
            inv = pltpu.reciprocal(den, approx=True)
            inv = inv * (2.0 - den * inv)
            for j in range(NJ):
                o_v[j, pl.ds(r0, AR), :] = inv * _sum(
                    [es[w] * v_v[j, pl.ds(HALO + r0 - DIL * w, AR), :] for w in range(W)])

    def route():
        r = _rb(r_v[...]) + 0.0
        tok = (lax.broadcasted_iota(jnp.int32, (RC, 128), 1) * RC
               + lax.broadcasted_iota(jnp.int32, (RC, 128), 0))
        bits = lax.bitcast_convert_type(r, jnp.int32)
        imin = -2 ** 31
        key = jnp.where(bits >= 0, bits, bits ^ 0x7FFFFFFF)
        key = jnp.where(r != r, imin + 1, key)
        sub = lax.broadcasted_iota(jnp.int32, (8, D), 0)
        xs = jnp.zeros((8, D), F32)
        gate = jnp.zeros((8, D), F32)
        for n in range(2):
            kmax = jnp.max(key, keepdims=True)
            hit = jnp.min(jnp.where(key == kmax, tok, S - 1), keepdims=True)
            rsel = jnp.sum(jnp.where(tok == hit, r, 0.0), keepdims=True)
            key = jnp.where(tok == hit, imin, key)
            idx = jnp.clip(hit[0, 0], 0, S - 1)
            idx_s[n] = idx
            xs = jnp.where(sub == n, _row(xn_v, idx, 1), xs)
            gate = jnp.where(sub == n, rsel, gate)
        xs_v[0] = xs
        xs_v[1] = _rb(jax.nn.sigmoid(gate))

    def ffn_pieces():
        wg, wu, wd = [r.bitcast(U32) for r in (wg_v, wu_v, wd_v)]
        xa, xb = xs_v[0, :, :D - 128], xs_v[0, :, D - 128:]
        ya, yb = jnp.zeros((8, D - 128), F32), jnp.zeros((8, 128), F32)
        hs = []
        for f0 in range(0, F, 512):
            nf = min(512, F - f0)
            gb = _nt(xb, _row(wg, f0, nf, LAST))
            yield
            ub = _nt(xb, _row(wu, f0, nf, LAST))
            yield
            h = []
            for c in range(0, nf, 128):
                nc = min(128, nf - c)
                g = _rb(gb[:, c:c + nc] + _nt(xa, _row(wg, f0 + c, nc, FIRST)))
                yield
                u = _rb(ub[:, c:c + nc] + _nt(xa, _row(wu, f0 + c, nc, FIRST)))
                h.append(_rb(_rb(_silu(g)) * u))
                yield
            hs.append(h)
        for f0, h in zip(range(0, F, 512), hs):
            for c, t in enumerate(h):
                ya += jnp.dot(t, _row(wd, f0 + c * 128, t.shape[1], FIRST), preferred_element_type=F32)
                yield
            yb += jnp.dot(jnp.concatenate(h, axis=1), _row(wd, f0, min(512, F - f0), LAST),
                          preferred_element_type=F32)
            yield
        y_v[...] = jnp.concatenate([ya, yb], axis=1)

    def scatter():
        y = _rb(_rb(y_v[...]) * xs_v[1])
        for n in range(2):
            idx = jnp.clip(idx_s[n], 0, S - 1)
            for j, t in enumerate(_tiles(y[n:n + 1])):
                xn_v[j, pl.ds(idx, 1), :] = _rb(xn_v[j, pl.ds(idx, 1), :] + t)

    def outproj(r0, nr):
        s = jnp.dot(_row(o_v, r0, nr), _row(wop_v, 0, D), preferred_element_type=F32)
        for c in range(0, nr, RC):
            xf = x_v[pl.ds(r0 + c, RC), :].astype(F32)
            out_v[pl.ds(r0 + c, RC), :] = (xf + s[c:c + RC] * _silu(_row(xn_v, r0 + c, RC))).astype(BF16)
        return _tiles(s)

    plan1, plan2, plan3, plan4 = PLANS[PLAN]
    done = {"attn": 0, "ln": 3 * T // RC}

    def side(pace, na, nl):
        attn(done["attn"], na, pace)
        ln(done["ln"], nl, pace)
        done["attn"] += na
        done["ln"] += nl

    def proj_region(plan):
        pace = Pacer()
        for i, p, na, nl in plan:
            pace.add(proj(i, p))
            side(pace, na, nl)

    def ffn_region():
        pace = Pacer()
        ffn = ffn_pieces()
        res, u = [], 0
        for i in range(5, 8):
            for r in proj_pieces(i):
                next(ffn, None)
                res += r
                if len(res) == NJ:
                    pace.add(res)
                    side(pace, plan3[u], 0)
                    if 2 <= u < 2 + NJ:
                        prep_wo(u - 2, pace)
                    res, u = [], u + 1
        scatter()

    def out_region():
        pace = Pacer()
        for n, na in enumerate(plan4):
            pace.add(outproj(*OUT_BLOCKS[n]))
            out_copy(n).start()
            side(pace, na, 0)

    def opaque_one():
        return (jnp.max(lax.bitcast_convert_type(r_v[...], jnp.int32)) | 1) & 1

    if ONLY >= 0:
        idx_s[2] = opaque_one()
        pl.when(idx_s[2] == 1)([lambda: proj_region(plan1), lambda: (proj_region(plan2), route())[0], ffn_region, out_region][ONLY])
        out_v[pl.ds(0, 16), pl.ds(0, D)] = (_row(o_v, idx_s[2], 16) + _row(xn_v, idx_s[2], 16) + _row(q_v, idx_s[2], 16) + _row(k_v, idx_s[2], 16) + _row(v_v, idx_s[2], 16) + xs_v[0, 0:1] + wop_v[0, pl.ds(idx_s[2], 16), 0:1].astype(F32)).astype(BF16)
        out_copy(0).start()
        out_copy(0).wait()
        return

    with scope("z0_pro"):
        for c in ([wr_copy(), x_copy(0)] + [wq_copy(kt) for kt in range(NJ)]
                  + [x_copy(1), wkv_copy(K), wkv_copy(V), x_copy(2), x_copy(3), wo_copy()]):
            c.start()
        r_v[...] = jnp.zeros_like(r_v)
        wr_copy().wait()
        x_copy(0).wait()
        ln(0, T // RC)
        idx_s[2] = opaque_one()
        for kts in ((0, 1, 2), (3, 4)):
            for kt in kts:
                wq_copy(kt).wait()
            prep_wqkv(Q, kts)
    with scope("z1_q0"):
        x_copy(1).wait()
        pace = Pacer()
        pace.add(proj(0, Q))
        ln(T // RC, T // RC, lambda x, f, lead: pace(x, f * 0.75, lead))
    with scope("z2_q1"):
        wkv_copy(K).wait()
        proj(1, Q)
        prep_wqkv(K)
    with scope("z3_k01"):
        wkv_copy(V).wait()
        x_copy(2).wait()
        pace = Pacer()
        pace.add(proj(0, K))
        prep_wqkv(V)
        pace.add(proj(1, K))
        ln(2 * T // RC, T // RC, pace)
    with scope("z4_r1"):
        x_copy(3).wait()
        for c in ffn_copies():
            c.start()
        proj_region(plan1)
    with scope("z5_r2"):
        wo_copy().wait()
        proj_region(plan2)
        route()
    with scope("z6_r3"):
        for c in ffn_copies():
            c.wait()
        ffn_region()
    with scope("z7_r4"):
        pl.when(idx_s[2] == 1)(out_region)
    with scope("z8_tail"):
        for n in range(len(OUT_BLOCKS)):
            out_copy(n).wait()
    assert done == {"attn": S // AR, "ln": S // RC}, done


@jax.jit
def pallas_recurrent_scan__sliding_local_dilated__moe_arch_mod__prompt_kernel(
    A_x, A_wqkv, A_wo, B_x, B_w_r, B_w_gate, B_w_up, B_w_down,
):
    hbm = pl.BlockSpec(memory_space=pltpu.HBM)
    vm = pltpu.VMEM
    dma = pltpu.SemaphoreType.DMA
    flags = {"XLA_TPU_EVENLY_DISTRIBUTE_CRITICAL_NODES": True} if LP else None
    out = pl.pallas_call(
        kernel,
        out_shape=jax.ShapeDtypeStruct((S, D), BF16),
        in_specs=[hbm] * 7,
        out_specs=hbm,
        scratch_shapes=[
            vm((S, D), BF16), vm((NJ, S, 128), F32),
            vm((NJ, S, 128), F32), vm((NJ, S + HALO, 128), F32), vm((NJ, S + HALO, 128), F32),
            vm((NJ, S, 128), F32), vm((S, D), BF16),
            vm((D,), BF16), vm((3, D, D), BF16), vm((NJ, 3 * D // 2, 128), U32), vm((D, D), BF16),
            vm((NJ, D // 2, 128), U32),
            vm((NJ, F, 128), BF16), vm((NJ, F, 128), BF16), vm((NJ, F, 128), BF16), vm((NJ, D, 128), F32),
            vm((RC, 128), F32), vm((2, 8, D), F32), vm((8, D), F32),
            pltpu.SMEM((3,), jnp.int32),
            dma((len(X_BLOCKS),)), dma((NJ + 4,)), dma((3, NJ)), dma((len(OUT_BLOCKS),)),
        ],
        compiler_params=pltpu.CompilerParams(vmem_limit_bytes=100 * 1024 * 1024, flags=flags),
    )(A_x.reshape(S, D), A_wqkv, A_wo, B_w_r, B_w_gate.T, B_w_up.T, B_w_down)
    return out.reshape(1, S, D)
```

```python
import numpy as np
import jax
import jax.numpy as jnp
from jax import lax
import jax.experimental.pallas as pl
import jax.experimental.pallas.tpu as pltpu

S, D, H, W, DIL, F = 2048, 640, 32, 8, 2, 1728
DH = D // H
NJ = D // 128
T = 256
HALO = 16
RC = 16
AR = 8
GA0 = 10
GA1 = 10
GA2 = 10
GA3 = 5
GL0 = 10
GL1 = 20
GLP = 20
LSP = 90
G2 = 5
KA = 3
FFN0 = 4
PLAN = 0
ONLY = -1
SCOPES = 0
G3 = 0
STG = 0
RXC = 1
WO0 = 4
M7 = 0
F4 = 1
LP = 0
F32, BF16, U32 = jnp.float32, jnp.bfloat16, jnp.uint32
EPS = 1.00135803e-05
SCALE = DH ** -0.5
NEG = -999292928.0
LOG2E = 1.4426950408889634
LOW, HIGH = np.uint32(0xFFFF), np.uint32(0xFFFF0000)
Q, K, V = 0, 1, 2
FIRST, LAST = range(NJ - 1), [NJ - 1]
X_BLOCKS = [(0, T), (T, T), (2 * T, T), (3 * T, S - 3 * T)]
WQ_BLOCKS = [(0, KA * 128), (KA * 128, D - KA * 128)]
OUT_BLOCKS = [(i * T, T) for i in range(7)] + [(7 * T, 128), (7 * T + 128, 64), (7 * T + 192, 64)]
PLANS = {
    0: ([(0, V, 0, 10), (1, V, 6, 8), (2, Q, 8, 8), (2, K, 8, 8), (2, V, 6, 6)],
        [(3, Q, 8, 7), (3, K, 8, 7), (3, V, 8, 7), (4, Q, 9, 7), (4, K, 9, 7), (4, V, 8, 5)],
        [12, 12, 11, 11, 11, 11, 11, 12, 12],
        [13, 13, 13, 13, 13, 10, 0, 0, 0, 0]),
    1: ([(0, V, 0, 10), (1, V, 7, 8), (2, Q, 9, 8), (2, K, 9, 8), (2, V, 7, 6)],
        [(3, Q, 9, 7), (3, K, 9, 7), (3, V, 9, 7), (4, Q, 9, 7), (4, K, 9, 7), (4, V, 9, 5)],
        [11, 11, 10, 10, 10, 10, 10, 12, 12],
        [13, 13, 13, 13, 12, 10, 0, 0, 0, 0]),
    3: ([(0, V, 0, 11), (1, V, 6, 9), (2, Q, 8, 9), (2, K, 8, 8), (2, V, 6, 6)],
        [(3, Q, 8, 8), (3, K, 8, 8), (3, V, 8, 8), (4, Q, 8, 8), (4, K, 7, 5)],
        [12, 12, 12, 11, 11, 11, 11, 11, 12, 11],
        [13, 13, 13, 13, 13, 10, 0, 0, 0, 0]),
    4: ([(0, V, 0, 11), (1, V, 6, 9), (2, Q, 8, 9), (2, K, 8, 8), (2, V, 6, 6)],
        [(3, Q, 8, 8), (3, K, 8, 8), (3, V, 8, 8), (4, Q, 8, 8), (4, K, 7, 5)],
        [13, 12, 11, 10, 10, 10, 10, 10, 11, 10],
        [14, 14, 14, 14, 14, 12, 0, 0, 0, 0]),
    5: ([(0, V, 0, 12), (1, V, 6, 10), (2, Q, 7, 10), (2, K, 7, 10), (2, V, 6, 6)],
        [(3, Q, 8, 9), (3, K, 8, 9), (3, V, 8, 9), (4, Q, 7, 5)],
        [13, 13, 12, 11, 11, 11, 11, 11, 11, 11, 10],
        [13, 13, 13, 13, 13, 9, 0, 0, 0, 0]),
    2: ([(0, V, 0, 12), (1, V, 6, 8), (2, Q, 8, 8), (2, K, 8, 8), (2, V, 6, 6)],
        [(3, Q, 8, 7), (3, K, 8, 7), (3, V, 8, 7), (4, Q, 8, 7), (4, K, 8, 6), (4, V, 7, 4)],
        [11, 11, 11, 11, 11, 11, 11, 11, 11],
        [14, 14, 14, 14, 13, 13, 0, 0, 0, 0]),
}


def _rb(x):
    return x.astype(BF16).astype(F32)


def _silu(z):
    h = 0.5 * z
    return h + h * jnp.tanh(h)


def _sum(t):
    a = t[0]
    for b in t[1:]:
        a = a + b
    return a


def _tiles(x):
    return [x[:, j * 128:(j + 1) * 128] for j in range(x.shape[1] // 128)]


def _words(x):
    return pltpu.bitcast(x, U32)


def _row(ref, r0, n, js=range(NJ)):
    if ref.dtype == U32:
        return jnp.concatenate([pltpu.bitcast(ref[j, pl.ds(r0 // 2, n // 2), :], BF16) for j in js], axis=1)
    return jnp.concatenate([ref[j, pl.ds(r0, n), :] for j in js], axis=1)


def _nn(a, b):
    return jnp.dot(a, b, preferred_element_type=F32)


def _nt(a, b):
    return lax.dot_general(a, b, (((1,), (1,)), ((), ())), preferred_element_type=F32)


class _NoScope:
    def __enter__(self):
        return self

    def __exit__(self, *a):
        return False


def scope(name):
    return jax.named_scope(name) if SCOPES else _NoScope()


def kernel(x_hbm, wqkv_hbm, wo_hbm, wr_hbm, wg_hbm, wu_hbm, wd_hbm, out_hbm,
           x_v, xn_v, q_v, k_v, v_v, o_v, out_v, wr_v, fence_v, wqkv_v, wt_v, wo_v, wop_v, wg_v, wu_v, wd_v, tmp_v,
           r_v, gate_v, y_v, idx_s, sem_in, sem_f, sem_o):
    def x_copy(n):
        r0, nr = X_BLOCKS[n]
        return pltpu.make_async_copy(x_hbm.at[pl.ds(r0, nr)], x_v.at[pl.ds(r0, nr)], sem_in.at[n])

    def wq_copy(n):
        rows = pl.ds(*WQ_BLOCKS[n])
        return pltpu.make_async_copy(wqkv_hbm.at[rows, pl.ds(0, D)], wqkv_v.at[Q, rows], sem_in.at[4 + n])

    def wkv_copy(p):
        return pltpu.make_async_copy(wqkv_hbm.at[:, pl.ds(p * D, D)], wqkv_v.at[p], sem_in.at[5 + p])

    def wo_copy():
        return pltpu.make_async_copy(wo_hbm, wo_v, sem_in.at[8])

    def wr_copy():
        return pltpu.make_async_copy(wr_hbm, wr_v, sem_in.at[9])

    def fence():
        return pltpu.make_async_copy(wr_hbm, fence_v, sem_in.at[10])

    def ffn_copies():
        return [pltpu.make_async_copy(src.at[:, pl.ds(j * 128, 128)], dst.at[j], sem_f.at[m, j])
                for m, (src, dst) in enumerate(((wg_hbm, wg_v), (wu_hbm, wu_v), (wd_hbm, wd_v))) for j in range(NJ)]

    def out_copy(n):
        r0, nr = OUT_BLOCKS[n]
        return pltpu.make_async_copy(out_v.at[pl.ds(r0, nr)], out_hbm.at[pl.ds(r0, nr)], sem_o.at[n])

    class Pacer:
        def __init__(self):
            self.tiles = []
            bits = lax.bitcast_convert_type(wr_v[...].astype(F32).reshape(1, D)[:, :128], jnp.int32)
            self.keep = jnp.broadcast_to(bits | 1, (AR, 128)) != 0

        def add(self, tiles):
            self.start = len(self.tiles)
            self.tiles += tiles

        def at(self, lead, span=1.0):
            def pace(x, frac, step=0.0):
                if step and x.shape[0] > AR:
                    return jnp.concatenate([pace(x[r:r + AR], frac + step * r / AR) for r in range(0, x.shape[0], AR)], axis=0)
                pos = self.start + frac * span * (len(self.tiles) - self.start) - lead / 10
                if pos < 0:
                    return x
                tile = self.tiles[min(int(pos), len(self.tiles) - 1)]
                r0 = int(pos % 1 * tile.shape[0]) // AR * AR
                return jnp.concatenate([jnp.where(self.keep, x[r:r + AR], tile[r0:r0 + AR])
                                        for r in range(0, x.shape[0], AR)], axis=0)
            return pace

    def no_pace(x, frac, step=0.0):
        return x

    def regroup(src, dst, row0):
        for dd in range(DH // 2):
            even = src[pl.ds(dd, H // 2, stride=DH), :]
            odd = src[pl.ds(dd + DH // 2, H // 2, stride=DH), :]
            r = (row0 + 2 * dd * H) // 2
            dst[pl.ds(r, H // 2), :] = (even & LOW) | (odd << 16)
            dst[pl.ds(r + H // 2, H // 2), :] = (even >> 16) | (odd & HIGH)

    def prep_wqkv(p, kts=range(NJ)):
        for kt in kts:
            tmp_v[kt] = _words(wqkv_v[p, pl.ds(kt * 128, 128), :].T)
        for kt in kts:
            regroup(tmp_v.at[kt], wt_v.at[kt], p * D)

    def prep_wo(j, pace):
        for r in range(0, D, 64):
            t = lax.bitcast_convert_type(_words(wo_v[pl.ds(r, 64), pl.ds(j * 128, 128)]), F32)
            tmp_v[j, pl.ds(r // 2, 32), :] = lax.bitcast_convert_type(pace(t, r / D / 2), U32)
        regroup(tmp_v.at[j], wop_v.at[j], 0)

    def ln(c0, n, pace1=no_pace, pace2=no_pace, pace3=no_pace):
        if n == 0:
            return
        wr = wr_v[...].astype(F32).reshape(1, D)
        lane = lax.broadcasted_iota(jnp.int32, (RC, 128), 1)
        racc = r_v[...]
        for c in range(c0, c0 + n):
            xf = x_v[pl.ds(c * RC, RC), :].astype(F32)
            mean = jnp.sum(pace1(_sum(_tiles(xf)), (c - c0) / n, STG / 100 / n), axis=-1, keepdims=True) * (1.0 / D)
            mb = _rb(mean)
            xc = xf - mb
            dm = mean - mb
            sq = jnp.sum(pace2(_sum(_tiles(xc * xc)), (c - c0) / n, STG / 100 / n), axis=-1, keepdims=True)
            var = jnp.maximum(sq * (1.0 / D) - dm * dm, 0.0)
            sd = _rb(jnp.sqrt(_rb(_rb(var) + EPS)))
            inv = pltpu.reciprocal(sd, full_range=False)
            if G3:
                inv = pace3(jnp.broadcast_to(inv, (RC, 128)), (c - c0) / n)
                inv = jnp.concatenate([inv] * NJ, axis=1)
            xn = _rb((_rb(xc) if RXC else xc) * inv)
            for j, t in enumerate(_tiles(xn)):
                xn_v[j, pl.ds(c * RC, RC), :] = t
            racc = jnp.where(lane == c, jnp.sum(xn * wr, axis=-1, keepdims=True), racc)
        r_v[...] = racc

    def qkv_tile(i, n):
        dst, off = [(q_v, 0), (k_v, HALO), (v_v, HALO)][n // NJ]
        return dst.at[n % NJ, pl.ds(off + i * T, T)]

    def proj(i, p, kts=range(NJ)):
        res = _tiles(_nt(_row(xn_v, i * T, T, kts), _row(wt_v, p * D, D, kts)))
        for j, t in enumerate(res):
            dst = qkv_tile(i, p * NJ + j)
            dst[...] = t if kts[0] == 0 else dst[...] + t
            if i == 0 and p != Q:
                (k_v, v_v)[p - K][j, pl.ds(0, HALO), :] = jnp.broadcast_to(t[0:1], (HALO, 128))
        return res

    def proj_pieces(i, n_first):
        for n0 in range(n_first, 3 * NJ, 4):
            ns = range(n0, min(n0 + 4, 3 * NJ))
            part = _nt(_row(xn_v, i * T, T, LAST), _row(wt_v, n0 * 128, len(ns) * 128, LAST))
            if len(ns) == 4 or not M7:
                yield []
            for n, t in zip(ns, _tiles(part)):
                res = t + _nt(_row(xn_v, i * T, T, FIRST), _row(wt_v, n * 128, 128, FIRST))
                qkv_tile(i, n)[...] = res
                yield [res]

    def attn(c0, n, pace):
        for c in range(c0, c0 + n):
            r0 = c * AR
            qs = [q_v[j, pl.ds(r0, AR), :] for j in range(NJ)]
            ls = []
            for w in range(W):
                a = _sum([qs[j] * k_v[j, pl.ds(HALO + r0 - DIL * w, AR), :] for j in range(NJ)])
                ls.append(pace(a, (c - c0 + w / W) / n))
            ls = [a + pltpu.roll(a, 64, 1) for a in ls]
            ls = [a + pltpu.roll(a, 32, 1) for a in ls]
            for w in range(W):
                if r0 < DIL * w:
                    pos = lax.broadcasted_iota(jnp.int32, (AR, 128), 0) + r0
                    ls[w] = jnp.where(pos >= DIL * w, ls[w], NEG / SCALE)
            mx = jnp.maximum
            m = mx(mx(mx(ls[0], ls[1]), mx(ls[2], ls[3])), mx(mx(ls[4], ls[5]), mx(ls[6], ls[7])))
            es = [jnp.exp2((l - m) * (SCALE * LOG2E)) for l in ls]
            den = _sum(es)
            inv = pltpu.reciprocal(den, approx=True)
            inv = inv * (2.0 - den * inv)
            for j in range(NJ):
                o_v[j, pl.ds(r0, AR), :] = inv * _sum(
                    [es[w] * v_v[j, pl.ds(HALO + r0 - DIL * w, AR), :] for w in range(W)])

    def route():
        r = _rb(r_v[...]) + 0.0
        tok = (lax.broadcasted_iota(jnp.int32, (RC, 128), 1) * RC
               + lax.broadcasted_iota(jnp.int32, (RC, 128), 0))
        bits = lax.bitcast_convert_type(r, jnp.int32)
        imin = -2 ** 31
        key = jnp.where(bits >= 0, bits, bits ^ 0x7FFFFFFF)
        key = jnp.where(r != r, imin + 1, key)
        sub = lax.broadcasted_iota(jnp.int32, (8, D), 0)
        xs = jnp.zeros((8, D), F32)
        gate = jnp.zeros((8, D), F32)
        for n in range(2):
            kmax = jnp.max(key, keepdims=True)
            hit = jnp.min(jnp.where(key == kmax, tok, S - 1), keepdims=True)
            rsel = jnp.sum(jnp.where(tok == hit, r, 0.0), keepdims=True)
            key = jnp.where(tok == hit, imin, key)
            idx = jnp.clip(hit[0, 0], 0, S - 1)
            idx_s[n] = idx
            xs = jnp.where(sub == n, _row(xn_v, idx, 1), xs)
            gate = jnp.where(sub == n, rsel, gate)
        gate_v[...] = _rb(jax.nn.sigmoid(gate))
        return xs

    def ffn_pieces():
        wg, wu, wd = [r.bitcast(U32) for r in (wg_v, wu_v, wd_v)]
        xs = route()
        for _ in range(FFN0):
            yield
        xa, xb = xs[:, :D - 128], xs[:, D - 128:]
        ya, yb = jnp.zeros((8, D - 128), F32), jnp.zeros((8, 128), F32)
        hs = []
        for f0 in range(0, F, 512):
            nf = min(512, F - f0)
            gb = _nt(xb, _row(wg, f0, nf, LAST))
            if nf > 256 or not F4:
                yield
            ub = _nt(xb, _row(wu, f0, nf, LAST))
            yield
            h = []
            for c in range(0, nf, 128):
                nc = min(128, nf - c)
                g = _rb(gb[:, c:c + nc] + _nt(xa, _row(wg, f0 + c, nc, FIRST)))
                yield
                u = _rb(ub[:, c:c + nc] + _nt(xa, _row(wu, f0 + c, nc, FIRST)))
                h.append(_rb(_rb(_silu(g)) * u))
                yield
            hs.append(h)
        for f0, h in zip(range(0, F, 512), hs):
            for c, t in enumerate(h):
                ya += _nn(t, _row(wd, f0 + c * 128, t.shape[1], FIRST))
                yield
            yb += _nn(jnp.concatenate(h, axis=1), _row(wd, f0, min(512, F - f0), LAST))
            yield
        y_v[...] = jnp.concatenate([ya, yb], axis=1)

    def scatter():
        y = _rb(_rb(y_v[...]) * gate_v[...])
        for n in range(2):
            idx = jnp.clip(idx_s[n], 0, S - 1)
            for j, t in enumerate(_tiles(y[n:n + 1])):
                xn_v[j, pl.ds(idx, 1), :] = _rb(xn_v[j, pl.ds(idx, 1), :] + t)

    def outproj(r0, nr):
        s = _nn(_row(o_v, r0, nr), _row(wop_v, 0, D))
        for c in range(0, nr, RC):
            xf = x_v[pl.ds(r0 + c, RC), :].astype(F32)
            out_v[pl.ds(r0 + c, RC), :] = (xf + s[c:c + RC] * _silu(_row(xn_v, r0 + c, RC))).astype(BF16)
        return _tiles(s)

    plan1, plan2, plan3, plan4 = PLANS[PLAN]
    done = {"attn": 0, "ln": 3 * T // RC}

    def side(pace, na, nl, ga, gl=0):
        attn(done["attn"], na, pace.at(ga))
        ln(done["ln"], nl, pace.at(gl), pace.at(gl - G2), pace.at(gl - G2 - G3))
        done["attn"] += na
        done["ln"] += nl

    def proj_region(plan, ga, gl):
        pace = Pacer()
        for i, p, na, nl in plan:
            pace.add(proj(i, p))
            side(pace, na, nl, ga, gl)

    def ffn_region():
        pace = Pacer()
        ffn = ffn_pieces()
        res, u = [], 0
        for i, n_first in [(4, (12 - len(plan3)) * NJ), (5, 0), (6, 0), (7, 0)]:
            for r in proj_pieces(i, n_first):
                next(ffn, None)
                res += r
                if len(res) == NJ:
                    pace.add(res)
                    side(pace, plan3[u], 0, GA2)
                    if WO0 <= u < WO0 + NJ:
                        prep_wo(u - WO0, pace.at(0))
                    res, u = [], u + 1
        for _ in ffn:
            pass
        scatter()

    def out_region():
        pace = Pacer()
        for n, na in enumerate(plan4):
            pace.add(outproj(*OUT_BLOCKS[n]))
            out_copy(n).start()
            side(pace, na, 0, GA3)

    def opaque_one():
        return (jnp.max(lax.bitcast_convert_type(r_v[...], jnp.int32)) | 1) & 1

    def sink():
        out_v[pl.ds(0, 16), pl.ds(0, D)] = (_row(o_v, idx_s[2], 16) + _row(xn_v, idx_s[2], 16) + _row(q_v, idx_s[2], 16) + _row(k_v, idx_s[2], 16) + _row(v_v, idx_s[2], 16) + wt_v[0, pl.ds(idx_s[2], 16), 0:1].astype(F32) + wop_v[0, pl.ds(idx_s[2], 16), 0:1].astype(F32)).astype(BF16)
        out_copy(0).start()
        out_copy(0).wait()

    if ONLY in (0, 1, 2, 3, 5):
        if ONLY >= 1:
            done["attn"] += sum(u[2] for u in plan1)
            done["ln"] += sum(u[3] for u in plan1)
        if ONLY >= 2:
            done["attn"] += sum(u[2] for u in plan2)
        if ONLY == 3:
            done["attn"] += sum(plan3)
        idx_s[2] = opaque_one()
        pl.when(idx_s[2] == 1)([lambda: proj_region(plan1, GA0, GL0), lambda: proj_region(plan2, GA1, GL1), ffn_region, out_region, None, lambda: (ffn_region(), out_region())[0]][ONLY])
        return sink()

    with scope("y0_wait"):
        for c in (wr_copy(), x_copy(0), x_copy(1), wq_copy(0), wq_copy(1), wkv_copy(K), wkv_copy(V),
                  x_copy(2), x_copy(3), wo_copy()):
            c.start()
        r_v[...] = jnp.zeros_like(r_v)
        wr_copy().wait()
        x_copy(0).wait()
    with scope("y1_ln0"):
        ln(0, T // RC)
    with scope("y2_ln1"):
        x_copy(1).wait()
        ln(T // RC, T // RC)
        if ONLY == 4:
            idx_s[2] = 1
    with scope("y3_prep"):
        wq_copy(0).wait()
        prep_wqkv(Q, range(KA))
    with scope("z1_qa"):
        wq_copy(1).wait()
        prep_wqkv(Q, range(KA, NJ))
        for i in range(2):
            proj(i, Q, range(KA))
    with scope("z2_qb"):
        wkv_copy(K).wait()
        prep_wqkv(K)
        for i in range(2):
            proj(i, Q, range(KA, NJ))
    with scope("z3_k01"):
        wkv_copy(V).wait()
        x_copy(2).wait()
        pace = Pacer()
        pace.add(proj(0, K))
        prep_wqkv(V)
        pace.add(proj(1, K))
        ln(2 * T // RC, T // RC, pace.at(GLP, LSP / 100), pace.at(GLP - G2, LSP / 100))
    if ONLY == 4:
        x_copy(3).wait()
        wo_copy().wait()
        return sink()
    with scope("z4_r1"):
        x_copy(3).wait()
        for c in ffn_copies():
            c.start()
        proj_region(plan1, GA0, GL0)
    with scope("z5_r2"):
        wo_copy().wait()
        fence().start()
        proj_region(plan2, GA1, GL1)
    with scope("z6_r3"):
        for c in ffn_copies():
            c.wait()
        ffn_region()
    with scope("z7_r4"):
        fence().wait()
        out_region()
    with scope("z8_tail"):
        for n in range(len(OUT_BLOCKS)):
            out_copy(n).wait()
    assert done == {"attn": S // AR, "ln": S // RC}, done


@jax.jit
def pallas_recurrent_scan__sliding_local_dilated__moe_arch_mod__prompt_kernel(
    A_x, A_wqkv, A_wo, B_x, B_w_r, B_w_gate, B_w_up, B_w_down,
):
    hbm = pl.BlockSpec(memory_space=pltpu.HBM)
    vm = pltpu.VMEM
    dma = pltpu.SemaphoreType.DMA
    flags = {"XLA_TPU_EVENLY_DISTRIBUTE_CRITICAL_NODES": True} if LP else None
    out = pl.pallas_call(
        kernel,
        out_shape=jax.ShapeDtypeStruct((S, D), BF16),
        in_specs=[hbm] * 7,
        out_specs=hbm,
        scratch_shapes=[
            vm((S, D), BF16), vm((NJ, S, 128), F32),
            vm((NJ, S, 128), F32), vm((NJ, S + HALO, 128), F32), vm((NJ, S + HALO, 128), F32),
            vm((NJ, S, 128), F32), vm((S, D), BF16),
            vm((D,), BF16), vm((D,), BF16), vm((3, D, D), BF16), vm((NJ, 3 * D // 2, 128), U32), vm((D, D), BF16),
            vm((NJ, D // 2, 128), U32),
            vm((NJ, F, 128), BF16), vm((NJ, F, 128), BF16), vm((NJ, F, 128), BF16), vm((NJ, D // 2, 128), U32),
            vm((RC, 128), F32), vm((8, D), F32), vm((8, D), F32),
            pltpu.SMEM((3,), jnp.int32),
            dma((11,)), dma((3, NJ)), dma((len(OUT_BLOCKS),)),
        ],
        compiler_params=pltpu.CompilerParams(vmem_limit_bytes=100 * 1024 * 1024, flags=flags),
    )(A_x.reshape(S, D), A_wqkv, A_wo, B_w_r, B_w_gate.T, B_w_up.T, B_w_down)
    return out.reshape(1, S, D)
```

```python
import numpy as np
import jax
import jax.numpy as jnp
from jax import lax
import jax.experimental.pallas as pl
import jax.experimental.pallas.tpu as pltpu

S, D, H, W, DIL, F = 2048, 640, 32, 8, 2, 1728
DH = D // H
NJ = D // 128
T = 256
HALO = 16
LR = 16
AR = 8
F32, BF16, U32 = jnp.float32, jnp.bfloat16, jnp.uint32
EPS = 1.00135803e-05
NEG = -999292928.0
SCALE = DH ** -0.5
LOG2E = 1.4426950408889634
LOW, HIGH = np.uint32(0xFFFF), np.uint32(0xFFFF0000)
Q, K, V = 0, 1, 2
FIRST, LAST = range(NJ - 1), [NJ - 1]

KA = 2
X_BLOCKS = [(0, T), (T, T), (2 * T, 2 * T), (4 * T, 4 * T)]
WQ_BLOCKS = [(0, KA * 128), (KA * 128, D - KA * 128)]
TAIL = 1
OUT_BLOCKS = [(i * T, T) for i in range(7)] + [
    [(7 * T, 128), (7 * T + 128, 64), (7 * T + 192, 64)],
    [(7 * T, 128), (7 * T + 128, 96), (7 * T + 224, 32)],
    [(7 * T, 192), (7 * T + 192, 64)],
    [(7 * T, 160), (7 * T + 160, 64), (7 * T + 224, 32)]][TAIL]

GLP = 10
G2P = 5
GA0 = 12
GL0 = 12
G20 = 6
GA1 = 15
GL1 = 15
G21 = 5
GA2 = 5
GA3 = 15
P0 = 2
P1 = 1
P2 = 1
P3 = 2
P4 = 1
PLAN0 = [(1, K, 0, [14, 12, 16, 15][P0]), (0, V, 0, [14, 16, 12, 13][P0])], (0, GLP, GLP - G2P)
PLAN1 = list(zip([1, 2, 2, 2], [V, Q, K, V], *[
    ([7, 7, 8, 6], [8, 7, 8, 5]), ([8, 7, 7, 6], [8, 8, 7, 5]), ([8, 7, 7, 6], [9, 7, 7, 5]),
    ([7, 7, 7, 7], [8, 8, 8, 4])][P1])), (GA0, GL0, GL0 - G20)
PLAN2 = list(zip([3, 3, 3, 4, 4, 4], [Q, K, V, Q, K, V], *[
    ([8, 8, 8, 9, 9, 8], [7, 7, 7, 7, 7, 5]), ([9, 8, 8, 9, 9, 7], [8, 7, 7, 7, 7, 4]),
    ([9, 9, 8, 8, 8, 8], [7, 7, 7, 8, 7, 4]), ([8, 9, 9, 8, 9, 7], [8, 7, 7, 7, 6, 5])][P2])), (GA1, GL1, GL1 - G21)
PLAN3 = [[12, 12, 11, 11, 11, 11, 11, 12, 12], [14, 12, 12, 12, 11, 11, 11, 10, 10],
         [13, 12, 12, 12, 11, 11, 11, 11, 10], [15, 12, 11, 11, 11, 11, 11, 11, 10]][P3], (GA2, 0, 0)
PLAN4 = [[13, 13, 13, 13, 13, 10, 0], [12, 12, 12, 12, 12, 15, 0],
         [14, 13, 12, 12, 12, 12, 0], [12, 12, 12, 11, 11, 11, 6]][P4], (GA3, 0, 0)
FFN_DELAY = 4
WO_FIRST = 4
FULL = 0
LP = 0


def _rb(x):
    return x.astype(BF16).astype(F32)


def _silu(z):
    h = 0.5 * z
    return h + h * jnp.tanh(h)


def _sum(terms):
    total = terms[0]
    for t in terms[1:]:
        total = total + t
    return total


def _tiles(x):
    return [x[:, j * 128:(j + 1) * 128] for j in range(x.shape[1] // 128)]


def _rows(ref, r0, n, js=range(NJ)):
    if ref.dtype == U32:
        return jnp.concatenate([pltpu.bitcast(ref[j, pl.ds(r0 // 2, n // 2), :], BF16) for j in js], axis=1)
    return jnp.concatenate([ref[j, pl.ds(r0, n), :] for j in js], axis=1)


def _nn(a, b):
    return jnp.dot(a, b, preferred_element_type=F32)


def _nt(a, b):
    return lax.dot_general(a, b, (((1,), (1,)), ((), ())), preferred_element_type=F32)


def _no_pace(x, frac):
    return x


class Pacer:
    def __init__(self, keep):
        self.keep = keep
        self.tiles = []
        self.start = 0

    def add(self, tiles):
        self.start = len(self.tiles)
        self.tiles += tiles

    def at(self, lead):
        def pace(x, frac):
            pos = self.start + frac * (len(self.tiles) - self.start) - lead / 10
            if pos < 0:
                return x
            tile = self.tiles[min(int(pos), len(self.tiles) - 1)]
            r0 = int(pos % 1 * tile.shape[0]) // AR * AR
            return jnp.concatenate([jnp.where(self.keep, x[r:r + AR], tile[r0:r0 + AR])
                                    for r in range(0, x.shape[0], AR)], axis=0)
        return pace


def _kernel(x_hbm, wqkv_hbm, wo_hbm, wr_hbm, wg_hbm, wu_hbm, wd_hbm, out_hbm,
            x_v, xn_v, q_v, k_v, v_v, o_v, out_v, wr_v, fence_v, wqkv_v, wt_v, wo_v, wop_v, wg_v, wu_v, wd_v,
            tmp_v, r_v, sem_in, sem_ffn, sem_out):
    def x_copy(n):
        rows = pl.ds(*X_BLOCKS[n])
        return pltpu.make_async_copy(x_hbm.at[rows], x_v.at[rows], sem_in.at[n])

    def wq_copy(n):
        rows = pl.ds(*WQ_BLOCKS[n])
        return pltpu.make_async_copy(wqkv_hbm.at[rows, pl.ds(0, D)], wqkv_v.at[Q, rows], sem_in.at[4 + n])

    def wkv_copy(p):
        return pltpu.make_async_copy(wqkv_hbm.at[:, pl.ds(p * D, D)], wqkv_v.at[p], sem_in.at[5 + p])

    def wo_copy():
        return pltpu.make_async_copy(wo_hbm, wo_v, sem_in.at[8])

    def wr_copy():
        return pltpu.make_async_copy(wr_hbm, wr_v, sem_in.at[9])

    def fence():
        return pltpu.make_async_copy(wr_hbm, fence_v, sem_in.at[10])

    def ffn_copies():
        return [pltpu.make_async_copy(src.at[:, pl.ds(j * 128, 128)], dst.at[j], sem_ffn.at[m, j])
                for m, (src, dst) in enumerate(((wg_hbm, wg_v), (wu_hbm, wu_v), (wd_hbm, wd_v)))
                for j in range(NJ)]

    def out_copy(n):
        rows = pl.ds(*OUT_BLOCKS[n])
        return pltpu.make_async_copy(out_v.at[rows], out_hbm.at[rows], sem_out.at[n])

    def router_weights():
        return wr_v[...].astype(F32).reshape(1, D)

    def new_pacer():
        bits = lax.bitcast_convert_type(router_weights()[:, :128], jnp.int32)
        return Pacer(jnp.broadcast_to(bits | 1, (AR, 128)) != 0)

    def regroup(src, dst, row0):
        for dd in range(DH // 2):
            even = src[pl.ds(dd, H // 2, stride=DH), :]
            odd = src[pl.ds(dd + DH // 2, H // 2, stride=DH), :]
            r = (row0 + 2 * dd * H) // 2
            dst[pl.ds(r, H // 2), :] = (even & LOW) | (odd << 16)
            dst[pl.ds(r + H // 2, H // 2), :] = (even >> 16) | (odd & HIGH)

    def prep_wqkv(p, kts=range(NJ)):
        for kt in kts:
            tmp_v[kt] = pltpu.bitcast(wqkv_v[p, pl.ds(kt * 128, 128), :].T, U32)
        for kt in kts:
            regroup(tmp_v.at[kt], wt_v.at[kt], p * D)

    def prep_wo(j, pace):
        for r in range(0, D, 64):
            words = pace(pltpu.bitcast(wo_v[pl.ds(r, 64), pl.ds(j * 128, 128)], F32), r / D / 2)
            tmp_v[j, pl.ds(r // 2, 32), :] = lax.bitcast_convert_type(words, U32)
        regroup(tmp_v.at[j], wop_v.at[j], 0)

    def layernorm(c0, n, pace1=_no_pace, pace2=_no_pace):
        if n == 0:
            return
        wr = router_weights()
        lane = lax.broadcasted_iota(jnp.int32, (LR, 128), 1)
        scores = r_v[...]
        for c in range(c0, c0 + n):
            x = x_v[pl.ds(c * LR, LR), :].astype(F32)
            mean = jnp.sum(pace1(_sum(_tiles(x)), (c - c0) / n), axis=-1, keepdims=True) * (1.0 / D)
            mean_b = _rb(mean)
            xc = x - mean_b
            shift = mean - mean_b
            sq = jnp.sum(pace2(_sum(_tiles(xc * xc)), (c - c0) / n), axis=-1, keepdims=True)
            var = jnp.maximum(sq * (1.0 / D) - shift * shift, 0.0)
            sd = _rb(jnp.sqrt(_rb(_rb(var) + EPS)))
            xn = _rb(_rb(xc) * (1.0 / sd if FULL else pltpu.reciprocal(sd, full_range=False)))
            for j, t in enumerate(_tiles(xn)):
                xn_v[j, pl.ds(c * LR, LR), :] = t
            scores = jnp.where(lane == c, jnp.sum(xn * wr, axis=-1, keepdims=True), scores)
        r_v[...] = scores

    def qkv_tile(i, n):
        dst, off = [(q_v, 0), (k_v, HALO), (v_v, HALO)][n // NJ]
        return dst.at[n % NJ, pl.ds(off + i * T, T)]

    def project(i, p, kts=range(NJ)):
        res = _tiles(_nt(_rows(xn_v, i * T, T, kts), _rows(wt_v, p * D, D, kts)))
        for j, t in enumerate(res):
            dst = qkv_tile(i, p * NJ + j)
            dst[...] = t if kts[0] == 0 else dst[...] + t
            if i == 0 and p != Q:
                (k_v, v_v)[p - K][j, pl.ds(0, HALO), :] = jnp.broadcast_to(t[0:1], (HALO, 128))
        return res

    def project_pieces(i):
        for n0 in range(0, 3 * NJ, 4):
            ns = range(n0, min(n0 + 4, 3 * NJ))
            part = _nt(_rows(xn_v, i * T, T, LAST), _rows(wt_v, n0 * 128, len(ns) * 128, LAST))
            yield []
            for n, t in zip(ns, _tiles(part)):
                res = t + _nt(_rows(xn_v, i * T, T, FIRST), _rows(wt_v, n * 128, 128, FIRST))
                qkv_tile(i, n)[...] = res
                yield [res]

    def attention(c0, n, pace):
        for c in range(c0, c0 + n):
            r0 = c * AR
            q = [q_v[j, pl.ds(r0, AR), :] for j in range(NJ)]
            ls = [pace(_sum([q[j] * k_v[j, pl.ds(HALO + r0 - DIL * w, AR), :] for j in range(NJ)]),
                       (c - c0 + w / W) / n) for w in range(W)]
            ls = [a + pltpu.roll(a, 2 * H, 1) for a in ls]
            ls = [a + pltpu.roll(a, H, 1) for a in ls]
            for w in range(W):
                if r0 < DIL * w:
                    pos = lax.broadcasted_iota(jnp.int32, (AR, 128), 0) + r0
                    ls[w] = jnp.where(pos >= DIL * w, ls[w], NEG / SCALE)
            mx = jnp.maximum
            top = mx(mx(mx(ls[0], ls[1]), mx(ls[2], ls[3])), mx(mx(ls[4], ls[5]), mx(ls[6], ls[7])))
            es = [jnp.exp2((a - top) * (SCALE * LOG2E)) for a in ls]
            den = _sum(es)
            inv = pltpu.reciprocal(den, approx=True)
            inv = inv * (2.0 - den * inv)
            for j in range(NJ):
                o_v[j, pl.ds(r0, AR), :] = inv * _sum(
                    [es[w] * v_v[j, pl.ds(HALO + r0 - DIL * w, AR), :] for w in range(W)])

    def route():
        r = _rb(r_v[...]) + 0.0
        row = (lax.broadcasted_iota(jnp.int32, (LR, 128), 1) * LR
               + lax.broadcasted_iota(jnp.int32, (LR, 128), 0))
        bits = lax.bitcast_convert_type(r, jnp.int32)
        taken = -2 ** 31
        key = jnp.where(r != r, taken + 1, jnp.where(bits >= 0, bits, bits ^ 0x7FFFFFFF))
        sub = lax.broadcasted_iota(jnp.int32, (8, D), 0)
        xs = jnp.zeros((8, D), F32)
        score = jnp.zeros((8, D), F32)
        picks = []
        for n in range(2):
            hit = jnp.min(jnp.where(key == jnp.max(key, keepdims=True), row, S - 1), keepdims=True)
            key = jnp.where(row == hit, taken, key)
            picks.append(jnp.clip(hit[0, 0], 0, S - 1))
            xs = jnp.where(sub == n, _rows(xn_v, picks[n], 1), xs)
            score = jnp.where(sub == n, jnp.sum(jnp.where(row == hit, r, 0.0), keepdims=True), score)
        return picks, xs, score

    def routed_pieces(result):
        wg, wu, wd = [ref.bitcast(U32) for ref in (wg_v, wu_v, wd_v)]
        picks, xs, score = route()
        for _ in range(FFN_DELAY):
            yield
        xa, xb = xs[:, :D - 128], xs[:, D - 128:]
        hidden = []
        for f0 in range(0, F, 512):
            nf = min(512, F - f0)
            gb = _nt(xb, _rows(wg, f0, nf, LAST))
            if nf == 512:
                yield
            ub = _nt(xb, _rows(wu, f0, nf, LAST))
            yield
            hs = []
            for c in range(0, nf, 128):
                nc = min(128, nf - c)
                g = _rb(gb[:, c:c + nc] + _nt(xa, _rows(wg, f0 + c, nc, FIRST)))
                yield
                u = _rb(ub[:, c:c + nc] + _nt(xa, _rows(wu, f0 + c, nc, FIRST)))
                hs.append(_rb(_rb(_silu(g)) * u))
                yield
            hidden.append((f0, nf, hs))
        ya, yb = jnp.zeros((8, D - 128), F32), jnp.zeros((8, 128), F32)
        for f0, nf, hs in hidden:
            for c, h in enumerate(hs):
                ya += _nn(h, _rows(wd, f0 + c * 128, h.shape[1], FIRST))
                yield
            yb += _nn(jnp.concatenate(hs, axis=1), _rows(wd, f0, nf, LAST))
            yield
        y = _rb(jnp.concatenate([ya, yb], axis=1))
        result.extend([picks, _rb(y * _rb(jax.nn.sigmoid(score)))])

    def output(r0, n):
        s = _nn(_rows(o_v, r0, n), _rows(wop_v, 0, D))
        for c in range(0, n, LR):
            x = x_v[pl.ds(r0 + c, LR), :].astype(F32)
            out_v[pl.ds(r0 + c, LR), :] = (x + s[c:c + LR] * _silu(_rows(xn_v, r0 + c, LR))).astype(BF16)
        return _tiles(s)

    done = {"attention": 0, "layernorm": 2 * T // LR}

    def side_work(pacer, na, nl, leads):
        attention(done["attention"], na, pacer.at(leads[0]))
        layernorm(done["layernorm"], nl, pacer.at(leads[1]), pacer.at(leads[2]))
        done["attention"] += na
        done["layernorm"] += nl

    def project_region(plan, leads):
        pacer = new_pacer()
        for i, p, na, nl in plan:
            pacer.add(project(i, p))
            side_work(pacer, na, nl, leads)

    def routed_region(plan, leads):
        pacer, result = new_pacer(), []
        routed = routed_pieces(result)
        res, unit = [], 0
        for i in range(5, S // T):
            for piece in project_pieces(i):
                next(routed, None)
                res += piece
                if len(res) == NJ:
                    pacer.add(res)
                    side_work(pacer, plan[unit], 0, leads)
                    if WO_FIRST <= unit < WO_FIRST + NJ:
                        prep_wo(unit - WO_FIRST, pacer.at(0))
                    res, unit = [], unit + 1
        for _ in routed:
            pass
        picks, update = result
        for n, idx in enumerate(picks):
            for j, t in enumerate(_tiles(update[n:n + 1])):
                xn_v[j, pl.ds(idx, 1), :] = _rb(xn_v[j, pl.ds(idx, 1), :] + t)

    def output_region(plan, leads):
        pacer = new_pacer()
        for n, block in enumerate(OUT_BLOCKS):
            pacer.add(output(*block))
            out_copy(n).start()
            if n < len(plan):
                side_work(pacer, plan[n], 0, leads)

    for copy in (wr_copy(), x_copy(0), wq_copy(0), x_copy(1), wq_copy(1), wkv_copy(K), wkv_copy(V),
                 x_copy(2), x_copy(3), wo_copy()):
        copy.start()
    r_v[...] = jnp.zeros_like(r_v)
    wr_copy().wait()
    x_copy(0).wait()
    layernorm(0, T // LR)
    wq_copy(0).wait()
    prep_wqkv(Q, range(KA))
    x_copy(1).wait()
    project(0, Q, range(KA))
    layernorm(T // LR, T // LR)
    wq_copy(1).wait()
    prep_wqkv(Q, range(KA, NJ))
    project(1, Q, range(KA))
    project(0, Q, range(KA, NJ))
    wkv_copy(K).wait()
    prep_wqkv(K)
    project(1, Q, range(KA, NJ))
    project(0, K)
    x_copy(2).wait()
    wkv_copy(V).wait()
    prep_wqkv(V)
    project_region(*PLAN0)

    x_copy(3).wait()
    for copy in ffn_copies():
        copy.start()
    project_region(*PLAN1)
    wo_copy().wait()
    fence().start()
    project_region(*PLAN2)
    for copy in ffn_copies():
        copy.wait()
    routed_region(*PLAN3)
    fence().wait()
    output_region(*PLAN4)
    for n in range(len(OUT_BLOCKS)):
        out_copy(n).wait()
    assert done == {"attention": S // AR, "layernorm": S // LR}


@jax.jit
def pallas_recurrent_scan__sliding_local_dilated__moe_arch_mod__prompt_kernel(
    A_x: jax.Array,
    A_wqkv: jax.Array,
    A_wo: jax.Array,
    B_x: jax.Array,
    B_w_r: jax.Array,
    B_w_gate: jax.Array,
    B_w_up: jax.Array,
    B_w_down: jax.Array,
):
    del B_x
    hbm = pl.BlockSpec(memory_space=pltpu.HBM)
    vmem = pltpu.VMEM
    dma = pltpu.SemaphoreType.DMA
    flags = {"XLA_TPU_EVENLY_DISTRIBUTE_CRITICAL_NODES": True} if LP else None
    out = pl.pallas_call(
        _kernel,
        out_shape=jax.ShapeDtypeStruct((S, D), BF16),
        in_specs=[hbm] * 7,
        out_specs=hbm,
        scratch_shapes=[
            vmem((S, D), BF16),
            vmem((NJ, S, 128), F32),
            vmem((NJ, S, 128), F32),
            vmem((NJ, HALO + S, 128), F32),
            vmem((NJ, HALO + S, 128), F32),
            vmem((NJ, S, 128), F32),
            vmem((S, D), BF16),
            vmem((D,), BF16),
            vmem((D,), BF16),
            vmem((3, D, D), BF16),
            vmem((NJ, 3 * D // 2, 128), U32),
            vmem((D, D), BF16),
            vmem((NJ, D // 2, 128), U32),
            vmem((NJ, F, 128), BF16),
            vmem((NJ, F, 128), BF16),
            vmem((NJ, F, 128), BF16),
            vmem((NJ, D // 2, 128), U32),
            vmem((LR, 128), F32),
            dma((11,)), dma((3, NJ)), dma((len(OUT_BLOCKS),)),
        ],
        compiler_params=pltpu.CompilerParams(vmem_limit_bytes=64 * 1024 * 1024, flags=flags),
    )(A_x.reshape(S, D), A_wqkv, A_wo, B_w_r, B_w_gate.T, B_w_up.T, B_w_down)
    return out.reshape(1, S, D)
```

```python
import numpy as np
import jax
import jax.numpy as jnp
from jax import lax
import jax.experimental.pallas as pl
import jax.experimental.pallas.tpu as pltpu

S, D, H, W, DIL, F = 2048, 640, 32, 8, 2, 1728
DH = D // H
NJ = D // 128
T = 256
HALO = 16
LR = 16
AR = 8
F32, BF16, U32 = jnp.float32, jnp.bfloat16, jnp.uint32
EPS = 1.00135803e-05
NEG = -999292928.0
SCALE = DH ** -0.5
LOG2E = 1.4426950408889634
LOW, HIGH = np.uint32(0xFFFF), np.uint32(0xFFFF0000)
Q, K, V = 0, 1, 2
FIRST, LAST = range(NJ - 1), [NJ - 1]

KA = 2
X_BLOCKS = [(0, T), (T, T), (2 * T, 2 * T), (4 * T, 4 * T)]
WQ_BLOCKS = [(0, KA * 128), (KA * 128, D - KA * 128)]
TAIL = 1
OUT_BLOCKS = [(i * T, T) for i in range(7)] + [
    [(7 * T, 128), (7 * T + 128, 64), (7 * T + 192, 64)],
    [(7 * T, 128), (7 * T + 128, 96), (7 * T + 224, 32)],
    [(7 * T, 192), (7 * T + 192, 64)],
    [(7 * T, 160), (7 * T + 160, 64), (7 * T + 224, 32)]][TAIL]

GLP = 12
G2P = 5
GA0 = 10
GL0 = 10
G20 = 4
GA1 = 15
GL1 = 15
G21 = 5
GA2 = 10
GA3 = 15
P0 = 2
P1 = 1
P2 = 1
P3 = 2
P4 = 1
PLAN0 = [(1, K, 0, [14, 12, 16, 15][P0]), (0, V, 0, [14, 16, 12, 13][P0])], (0, GLP, GLP - G2P)
PLAN1 = list(zip([1, 2, 2, 2], [V, Q, K, V], *[
    ([7, 7, 8, 6], [8, 7, 8, 5]), ([8, 7, 7, 6], [8, 8, 7, 5]), ([8, 7, 7, 6], [9, 7, 7, 5]),
    ([7, 7, 7, 7], [8, 8, 8, 4])][P1])), (GA0, GL0, GL0 - G20)
PLAN2 = list(zip([3, 3, 3, 4, 4, 4], [Q, K, V, Q, K, V], *[
    ([8, 8, 8, 9, 9, 8], [7, 7, 7, 7, 7, 5]), ([9, 8, 8, 9, 9, 7], [8, 7, 7, 7, 7, 4]),
    ([9, 9, 8, 8, 8, 8], [7, 7, 7, 8, 7, 4]), ([8, 9, 9, 8, 9, 7], [8, 7, 7, 7, 6, 5])][P2])), (GA1, GL1, GL1 - G21)
PLAN3 = [[12, 12, 11, 11, 11, 11, 11, 12, 12], [14, 12, 12, 12, 11, 11, 11, 10, 10],
         [13, 12, 12, 12, 11, 11, 11, 11, 10], [15, 12, 11, 11, 11, 11, 11, 11, 10]][P3], (GA2, 0, 0)
PLAN4 = [[13, 13, 13, 13, 13, 10, 0], [12, 12, 12, 12, 12, 15, 0],
         [14, 13, 12, 12, 12, 12, 0], [12, 12, 12, 11, 11, 11, 6]][P4], (GA3, 0, 0)
FFN_DELAY = 4
WO_FIRST = 4
FULL = 0
LP = 0


def _rb(x):
    return x.astype(BF16).astype(F32)


def _silu(z):
    h = 0.5 * z
    return h + h * jnp.tanh(h)


def _sum(terms):
    total = terms[0]
    for t in terms[1:]:
        total = total + t
    return total


def _tiles(x):
    return [x[:, j * 128:(j + 1) * 128] for j in range(x.shape[1] // 128)]


def _rows(ref, r0, n, js=range(NJ)):
    if ref.dtype == U32:
        return jnp.concatenate([pltpu.bitcast(ref[j, pl.ds(r0 // 2, n // 2), :], BF16) for j in js], axis=1)
    return jnp.concatenate([ref[j, pl.ds(r0, n), :] for j in js], axis=1)


def _nn(a, b):
    return jnp.dot(a, b, preferred_element_type=F32)


def _nt(a, b):
    return lax.dot_general(a, b, (((1,), (1,)), ((), ())), preferred_element_type=F32)


def _no_pace(x, frac):
    return x


class Pacer:
    def __init__(self, keep):
        self.keep = keep
        self.tiles = []
        self.start = 0

    def add(self, tiles):
        self.start = len(self.tiles)
        self.tiles += tiles

    def at(self, lead):
        def pace(x, frac):
            pos = self.start + frac * (len(self.tiles) - self.start) - lead / 10
            if pos < 0:
                return x
            tile = self.tiles[min(int(pos), len(self.tiles) - 1)]
            r0 = int(pos % 1 * tile.shape[0]) // AR * AR
            return jnp.concatenate([jnp.where(self.keep, x[r:r + AR], tile[r0:r0 + AR])
                                    for r in range(0, x.shape[0], AR)], axis=0)
        return pace


def _kernel(x_hbm, wqkv_hbm, wo_hbm, wr_hbm, wg_hbm, wu_hbm, wd_hbm, out_hbm,
            x_v, xn_v, q_v, k_v, v_v, o_v, out_v, wr_v, fence_v, wqkv_v, wt_v, wo_v, wop_v, wg_v, wu_v, wd_v,
            tmp_v, r_v, sem_in, sem_ffn, sem_out):
    def x_copy(n):
        rows = pl.ds(*X_BLOCKS[n])
        return pltpu.make_async_copy(x_hbm.at[rows], x_v.at[rows], sem_in.at[n])

    def wq_copy(n):
        rows = pl.ds(*WQ_BLOCKS[n])
        return pltpu.make_async_copy(wqkv_hbm.at[rows, pl.ds(0, D)], wqkv_v.at[Q, rows], sem_in.at[4 + n])

    def wkv_copy(p):
        return pltpu.make_async_copy(wqkv_hbm.at[:, pl.ds(p * D, D)], wqkv_v.at[p], sem_in.at[5 + p])

    def wo_copy():
        return pltpu.make_async_copy(wo_hbm, wo_v, sem_in.at[8])

    def wr_copy():
        return pltpu.make_async_copy(wr_hbm, wr_v, sem_in.at[9])

    def fence():
        return pltpu.make_async_copy(wr_hbm, fence_v, sem_in.at[10])

    def ffn_copies():
        return [pltpu.make_async_copy(src.at[:, pl.ds(j * 128, 128)], dst.at[j], sem_ffn.at[m, j])
                for m, (src, dst) in enumerate(((wg_hbm, wg_v), (wu_hbm, wu_v), (wd_hbm, wd_v)))
                for j in range(NJ)]

    def out_copy(n):
        rows = pl.ds(*OUT_BLOCKS[n])
        return pltpu.make_async_copy(out_v.at[rows], out_hbm.at[rows], sem_out.at[n])

    def router_weights():
        return wr_v[...].astype(F32).reshape(1, D)

    def new_pacer():
        bits = lax.bitcast_convert_type(router_weights()[:, :128], jnp.int32)
        return Pacer(jnp.broadcast_to(bits | 1, (AR, 128)) != 0)

    def regroup(src, dst, row0):
        for dd in range(DH // 2):
            even = src[pl.ds(dd, H // 2, stride=DH), :]
            odd = src[pl.ds(dd + DH // 2, H // 2, stride=DH), :]
            r = (row0 + 2 * dd * H) // 2
            dst[pl.ds(r, H // 2), :] = (even & LOW) | (odd << 16)
            dst[pl.ds(r + H // 2, H // 2), :] = (even >> 16) | (odd & HIGH)

    def prep_wqkv(p, kts=range(NJ)):
        for kt in kts:
            tmp_v[kt] = pltpu.bitcast(wqkv_v[p, pl.ds(kt * 128, 128), :].T, U32)
        for kt in kts:
            regroup(tmp_v.at[kt], wt_v.at[kt], p * D)

    def prep_wo(j, pace):
        for r in range(0, D, 64):
            words = pace(pltpu.bitcast(wo_v[pl.ds(r, 64), pl.ds(j * 128, 128)], F32), r / D / 2)
            tmp_v[j, pl.ds(r // 2, 32), :] = lax.bitcast_convert_type(words, U32)
        regroup(tmp_v.at[j], wop_v.at[j], 0)

    def layernorm(c0, n, pace1=_no_pace, pace2=_no_pace):
        if n == 0:
            return
        wr = router_weights()
        lane = lax.broadcasted_iota(jnp.int32, (LR, 128), 1)
        scores = r_v[...]
        for c in range(c0, c0 + n):
            x = x_v[pl.ds(c * LR, LR), :].astype(F32)
            mean = jnp.sum(pace1(_sum(_tiles(x)), (c - c0) / n), axis=-1, keepdims=True) * (1.0 / D)
            mean_b = _rb(mean)
            xc = x - mean_b
            shift = mean - mean_b
            sq = jnp.sum(pace2(_sum(_tiles(xc * xc)), (c - c0) / n), axis=-1, keepdims=True)
            var = jnp.maximum(sq * (1.0 / D) - shift * shift, 0.0)
            sd = _rb(jnp.sqrt(_rb(_rb(var) + EPS)))
            xn = _rb(_rb(xc) * (1.0 / sd if FULL else pltpu.reciprocal(sd, full_range=False)))
            for j, t in enumerate(_tiles(xn)):
                xn_v[j, pl.ds(c * LR, LR), :] = t
            scores = jnp.where(lane == c, jnp.sum(xn * wr, axis=-1, keepdims=True), scores)
        r_v[...] = scores

    def qkv_tile(i, n):
        dst, off = [(q_v, 0), (k_v, HALO), (v_v, HALO)][n // NJ]
        return dst.at[n % NJ, pl.ds(off + i * T, T)]

    def project(i, p, kts=range(NJ)):
        res = _tiles(_nt(_rows(xn_v, i * T, T, kts), _rows(wt_v, p * D, D, kts)))
        for j, t in enumerate(res):
            dst = qkv_tile(i, p * NJ + j)
            dst[...] = t if kts[0] == 0 else dst[...] + t
            if i == 0 and p != Q:
                (k_v, v_v)[p - K][j, pl.ds(0, HALO), :] = jnp.broadcast_to(t[0:1], (HALO, 128))
        return res

    def project_pieces(i):
        for n0 in range(0, 3 * NJ, 4):
            ns = range(n0, min(n0 + 4, 3 * NJ))
            part = _nt(_rows(xn_v, i * T, T, LAST), _rows(wt_v, n0 * 128, len(ns) * 128, LAST))
            yield []
            for n, t in zip(ns, _tiles(part)):
                res = t + _nt(_rows(xn_v, i * T, T, FIRST), _rows(wt_v, n * 128, 128, FIRST))
                qkv_tile(i, n)[...] = res
                yield [res]

    def attention(c0, n, pace):
        for c in range(c0, c0 + n):
            r0 = c * AR
            q = [q_v[j, pl.ds(r0, AR), :] for j in range(NJ)]
            ls = [pace(_sum([q[j] * k_v[j, pl.ds(HALO + r0 - DIL * w, AR), :] for j in range(NJ)]),
                       (c - c0 + w / W) / n) for w in range(W)]
            ls = [a + pltpu.roll(a, 2 * H, 1) for a in ls]
            ls = [a + pltpu.roll(a, H, 1) for a in ls]
            for w in range(W):
                if r0 < DIL * w:
                    pos = lax.broadcasted_iota(jnp.int32, (AR, 128), 0) + r0
                    ls[w] = jnp.where(pos >= DIL * w, ls[w], NEG / SCALE)
            mx = jnp.maximum
            top = mx(mx(mx(ls[0], ls[1]), mx(ls[2], ls[3])), mx(mx(ls[4], ls[5]), mx(ls[6], ls[7])))
            es = [jnp.exp2((a - top) * (SCALE * LOG2E)) for a in ls]
            den = _sum(es)
            inv = pltpu.reciprocal(den, approx=True)
            inv = inv * (2.0 - den * inv)
            for j in range(NJ):
                o_v[j, pl.ds(r0, AR), :] = inv * _sum(
                    [es[w] * v_v[j, pl.ds(HALO + r0 - DIL * w, AR), :] for w in range(W)])

    def route():
        r = _rb(r_v[...]) + 0.0
        row = (lax.broadcasted_iota(jnp.int32, (LR, 128), 1) * LR
               + lax.broadcasted_iota(jnp.int32, (LR, 128), 0))
        bits = lax.bitcast_convert_type(r, jnp.int32)
        taken = -2 ** 31
        key = jnp.where(r != r, taken + 1, jnp.where(bits >= 0, bits, bits ^ 0x7FFFFFFF))
        sub = lax.broadcasted_iota(jnp.int32, (8, D), 0)
        xs = jnp.zeros((8, D), F32)
        score = jnp.zeros((8, D), F32)
        picks = []
        for n in range(2):
            hit = jnp.min(jnp.where(key == jnp.max(key, keepdims=True), row, S - 1), keepdims=True)
            key = jnp.where(row == hit, taken, key)
            picks.append(jnp.clip(hit[0, 0], 0, S - 1))
            xs = jnp.where(sub == n, _rows(xn_v, picks[n], 1), xs)
            score = jnp.where(sub == n, jnp.sum(jnp.where(row == hit, r, 0.0), keepdims=True), score)
        return picks, xs, score

    def routed_pieces(result):
        wg, wu, wd = [ref.bitcast(U32) for ref in (wg_v, wu_v, wd_v)]
        picks, xs, score = route()
        for _ in range(FFN_DELAY):
            yield
        xa, xb = xs[:, :D - 128], xs[:, D - 128:]
        hidden = []
        for f0 in range(0, F, 512):
            nf = min(512, F - f0)
            gb = _nt(xb, _rows(wg, f0, nf, LAST))
            if nf == 512:
                yield
            ub = _nt(xb, _rows(wu, f0, nf, LAST))
            yield
            hs = []
            for c in range(0, nf, 128):
                nc = min(128, nf - c)
                g = _rb(gb[:, c:c + nc] + _nt(xa, _rows(wg, f0 + c, nc, FIRST)))
                yield
                u = _rb(ub[:, c:c + nc] + _nt(xa, _rows(wu, f0 + c, nc, FIRST)))
                hs.append(_rb(_rb(_silu(g)) * u))
                yield
            hidden.append((f0, nf, hs))
        ya, yb = jnp.zeros((8, D - 128), F32), jnp.zeros((8, 128), F32)
        for f0, nf, hs in hidden:
            for c, h in enumerate(hs):
                ya += _nn(h, _rows(wd, f0 + c * 128, h.shape[1], FIRST))
                yield
            yb += _nn(jnp.concatenate(hs, axis=1), _rows(wd, f0, nf, LAST))
            yield
        y = _rb(jnp.concatenate([ya, yb], axis=1))
        result.extend([picks, _rb(y * _rb(jax.nn.sigmoid(score)))])

    def output(r0, n):
        s = _nn(_rows(o_v, r0, n), _rows(wop_v, 0, D))
        for c in range(0, n, LR):
            x = x_v[pl.ds(r0 + c, LR), :].astype(F32)
            out_v[pl.ds(r0 + c, LR), :] = (x + s[c:c + LR] * _silu(_rows(xn_v, r0 + c, LR))).astype(BF16)
        return _tiles(s)

    done = {"attention": 0, "layernorm": 2 * T // LR}

    def side_work(pacer, na, nl, leads):
        attention(done["attention"], na, pacer.at(leads[0]))
        layernorm(done["layernorm"], nl, pacer.at(leads[1]), pacer.at(leads[2]))
        done["attention"] += na
        done["layernorm"] += nl

    def project_region(plan, leads):
        pacer = new_pacer()
        for i, p, na, nl in plan:
            pacer.add(project(i, p))
            side_work(pacer, na, nl, leads)

    def routed_region(plan, leads):
        pacer, result = new_pacer(), []
        routed = routed_pieces(result)
        res, unit = [], 0
        for i in range(5, S // T):
            for piece in project_pieces(i):
                next(routed, None)
                res += piece
                if len(res) == NJ:
                    pacer.add(res)
                    side_work(pacer, plan[unit], 0, leads)
                    if WO_FIRST <= unit < WO_FIRST + NJ:
                        prep_wo(unit - WO_FIRST, pacer.at(0))
                    res, unit = [], unit + 1
        for _ in routed:
            pass
        picks, update = result
        for n, idx in enumerate(picks):
            for j, t in enumerate(_tiles(update[n:n + 1])):
                xn_v[j, pl.ds(idx, 1), :] = _rb(xn_v[j, pl.ds(idx, 1), :] + t)

    def output_region(plan, leads):
        pacer = new_pacer()
        for n, block in enumerate(OUT_BLOCKS):
            pacer.add(output(*block))
            out_copy(n).start()
            if n < len(plan):
                side_work(pacer, plan[n], 0, leads)

    for copy in (wr_copy(), x_copy(0), wq_copy(0), x_copy(1), wq_copy(1), wkv_copy(K), wkv_copy(V),
                 x_copy(2), x_copy(3), wo_copy()):
        copy.start()
    r_v[...] = jnp.zeros_like(r_v)
    wr_copy().wait()
    x_copy(0).wait()
    layernorm(0, T // LR)
    wq_copy(0).wait()
    prep_wqkv(Q, range(KA))
    x_copy(1).wait()
    project(0, Q, range(KA))
    layernorm(T // LR, T // LR)
    wq_copy(1).wait()
    prep_wqkv(Q, range(KA, NJ))
    project(1, Q, range(KA))
    project(0, Q, range(KA, NJ))
    wkv_copy(K).wait()
    prep_wqkv(K)
    project(1, Q, range(KA, NJ))
    project(0, K)
    x_copy(2).wait()
    wkv_copy(V).wait()
    prep_wqkv(V)
    project_region(*PLAN0)

    x_copy(3).wait()
    for copy in ffn_copies():
        copy.start()
    project_region(*PLAN1)
    wo_copy().wait()
    fence().start()
    project_region(*PLAN2)
    for copy in ffn_copies():
        copy.wait()
    routed_region(*PLAN3)
    fence().wait()
    output_region(*PLAN4)
    for n in range(len(OUT_BLOCKS)):
        out_copy(n).wait()
    assert done == {"attention": S // AR, "layernorm": S // LR}


@jax.jit
def pallas_recurrent_scan__sliding_local_dilated__moe_arch_mod__prompt_kernel(
    A_x: jax.Array,
    A_wqkv: jax.Array,
    A_wo: jax.Array,
    B_x: jax.Array,
    B_w_r: jax.Array,
    B_w_gate: jax.Array,
    B_w_up: jax.Array,
    B_w_down: jax.Array,
):
    del B_x
    hbm = pl.BlockSpec(memory_space=pltpu.HBM)
    vmem = pltpu.VMEM
    dma = pltpu.SemaphoreType.DMA
    flags = {"XLA_TPU_EVENLY_DISTRIBUTE_CRITICAL_NODES": True} if LP else None
    out = pl.pallas_call(
        _kernel,
        out_shape=jax.ShapeDtypeStruct((S, D), BF16),
        in_specs=[hbm] * 7,
        out_specs=hbm,
        scratch_shapes=[
            vmem((S, D), BF16),
            vmem((NJ, S, 128), F32),
            vmem((NJ, S, 128), F32),
            vmem((NJ, HALO + S, 128), F32),
            vmem((NJ, HALO + S, 128), F32),
            vmem((NJ, S, 128), F32),
            vmem((S, D), BF16),
            vmem((D,), BF16),
            vmem((D,), BF16),
            vmem((3, D, D), BF16),
            vmem((NJ, 3 * D // 2, 128), U32),
            vmem((D, D), BF16),
            vmem((NJ, D // 2, 128), U32),
            vmem((NJ, F, 128), BF16),
            vmem((NJ, F, 128), BF16),
            vmem((NJ, F, 128), BF16),
            vmem((NJ, D // 2, 128), U32),
            vmem((LR, 128), F32),
            dma((11,)), dma((3, NJ)), dma((len(OUT_BLOCKS),)),
        ],
        compiler_params=pltpu.CompilerParams(vmem_limit_bytes=64 * 1024 * 1024, flags=flags),
    )(A_x.reshape(S, D), A_wqkv, A_wo, B_w_r, B_w_gate.T, B_w_up.T, B_w_down)
    return out.reshape(1, S, D)
```

```python
import numpy as np
import jax
import jax.numpy as jnp
from jax import lax
import jax.experimental.pallas as pl
import jax.experimental.pallas.tpu as pltpu

S, D, H, W, DIL, F = 2048, 640, 32, 8, 2, 1728
DH = D // H
NJ = D // 128
T = 256
HALO = 16
LR = 16
AR = 8
F32, BF16, U32 = jnp.float32, jnp.bfloat16, jnp.uint32
EPS = 1.00135803e-05
NEG = -999292928.0
SCALE = DH ** -0.5
LOG2E = 1.4426950408889634
LOW, HIGH = np.uint32(0xFFFF), np.uint32(0xFFFF0000)
Q, K, V = 0, 1, 2
FIRST, LAST = range(NJ - 1), [NJ - 1]

KA = 2
X_BLOCKS = [(0, T), (T, T), (2 * T, 2 * T), (4 * T, 4 * T)]
WQ_BLOCKS = [(0, KA * 128), (KA * 128, D - KA * 128)]
OUT_BLOCKS = [(i * T, T) for i in range(7)] + [(7 * T, 128), (7 * T + 128, 96), (7 * T + 224, 32)]

PLAN_FIRST = [(0, Q, 0, 16)], (0, 50, 15)
PLAN0 = [(1, K, 0, 16), (0, V, 0, 12)], (0, 12, 7)
PLAN1 = [(1, V, 8, 8), (2, Q, 7, 8), (2, K, 7, 7), (2, V, 6, 5)], (10, 10, 6)
PLAN2 = [(3, Q, 9, 8), (3, K, 8, 7), (3, V, 8, 7), (4, Q, 9, 7), (4, K, 9, 7), (4, V, 7, 4)], (15, 15, 10)
PLAN3 = [13, 11, 11, 11, 10, 10, 10, 11, 10], (10, 0, 0)
PLAN4 = [12, 12, 12, 12, 12, 13, 8], (15, 0, 0)
FFN_DELAY = 4
WO_FIRST = 3


def _rb(x):
    return x.astype(BF16).astype(F32)


def _silu(z):
    h = 0.5 * z
    return h + h * jnp.tanh(h)


def _sum(terms):
    total = terms[0]
    for t in terms[1:]:
        total = total + t
    return total


def _tiles(x):
    return [x[:, j * 128:(j + 1) * 128] for j in range(x.shape[1] // 128)]


def _rows(ref, r0, n, js=range(NJ)):
    if ref.dtype == U32:
        return jnp.concatenate([pltpu.bitcast(ref[j, pl.ds(r0 // 2, n // 2), :], BF16) for j in js], axis=1)
    return jnp.concatenate([ref[j, pl.ds(r0, n), :] for j in js], axis=1)


def _nn(a, b):
    return jnp.dot(a, b, preferred_element_type=F32)


def _nt(a, b):
    return lax.dot_general(a, b, (((1,), (1,)), ((), ())), preferred_element_type=F32)


def _no_pace(x, frac):
    return x


class Pacer:
    def __init__(self, keep):
        self.keep = keep
        self.tiles = []
        self.start = 0

    def add(self, tiles):
        self.start = len(self.tiles)
        self.tiles += tiles

    def at(self, lead):
        def pace(x, frac):
            pos = self.start + frac * (len(self.tiles) - self.start) - lead / 10
            if pos < 0:
                return x
            tile = self.tiles[min(int(pos), len(self.tiles) - 1)]
            r0 = int(pos % 1 * tile.shape[0]) // AR * AR
            return jnp.concatenate([jnp.where(self.keep, x[r:r + AR], tile[r0:r0 + AR])
                                    for r in range(0, x.shape[0], AR)], axis=0)
        return pace


def _kernel(x_hbm, wqkv_hbm, wo_hbm, wr_hbm, wg_hbm, wu_hbm, wd_hbm, out_hbm,
            x_v, xn_v, q_v, k_v, v_v, o_v, out_v, wr_v, fence_v, wqkv_v, wt_v, wo_v, wop_v, wg_v, wu_v, wd_v,
            tmp_v, r_v, sem_in, sem_out):
    def x_copy(n):
        rows = pl.ds(*X_BLOCKS[n])
        return pltpu.make_async_copy(x_hbm.at[rows], x_v.at[rows], sem_in.at[n])

    def wq_copy(n):
        rows = pl.ds(*WQ_BLOCKS[n])
        return pltpu.make_async_copy(wqkv_hbm.at[rows, pl.ds(0, D)], wqkv_v.at[Q, rows], sem_in.at[4 + n])

    def wkv_copy(p):
        return pltpu.make_async_copy(wqkv_hbm.at[:, pl.ds(p * D, D)], wqkv_v.at[p], sem_in.at[5 + p])

    def wo_copy():
        return pltpu.make_async_copy(wo_hbm, wo_v, sem_in.at[8])

    def wr_copy():
        return pltpu.make_async_copy(wr_hbm, wr_v, sem_in.at[9])

    def fence():
        return pltpu.make_async_copy(wr_hbm, fence_v, sem_in.at[10])

    def ffn_copies():
        return [pltpu.make_async_copy(src, dst, sem_in.at[11 + m])
                for m, (src, dst) in enumerate(((wg_hbm, wg_v), (wu_hbm, wu_v), (wd_hbm, wd_v)))]

    def out_copy(n):
        rows = pl.ds(*OUT_BLOCKS[n])
        return pltpu.make_async_copy(out_v.at[rows], out_hbm.at[rows], sem_out.at[n])

    def router_weights():
        return wr_v[...].astype(F32).reshape(1, D)

    def new_pacer():
        bits = lax.bitcast_convert_type(router_weights()[:, :128], jnp.int32)
        return Pacer(jnp.broadcast_to(bits | 1, (AR, 128)) != 0)

    def regroup(src, dst, row0):
        for dd in range(DH // 2):
            even = src[pl.ds(dd, H // 2, stride=DH), :]
            odd = src[pl.ds(dd + DH // 2, H // 2, stride=DH), :]
            r = (row0 + 2 * dd * H) // 2
            dst[pl.ds(r, H // 2), :] = (even & LOW) | (odd << 16)
            dst[pl.ds(r + H // 2, H // 2), :] = (even >> 16) | (odd & HIGH)

    def prep_wqkv(p, kts=range(NJ)):
        for kt in kts:
            tmp_v[kt] = pltpu.bitcast(wqkv_v[p, pl.ds(kt * 128, 128), :].T, U32)
        for kt in kts:
            regroup(tmp_v.at[kt], wt_v.at[kt], p * D)

    def prep_wo(j, pace):
        for r in range(0, D, 64):
            words = pace(pltpu.bitcast(wo_v[pl.ds(r, 64), pl.ds(j * 128, 128)], F32), r / D / 2)
            tmp_v[j, pl.ds(r // 2, 32), :] = lax.bitcast_convert_type(words, U32)
        regroup(tmp_v.at[j], wop_v.at[j], 0)

    def layernorm(c0, n, pace1=_no_pace, pace2=_no_pace):
        if n == 0:
            return
        wr = router_weights()
        lane = lax.broadcasted_iota(jnp.int32, (LR, 128), 1)
        scores = r_v[...]
        for c in range(c0, c0 + n):
            x = x_v[pl.ds(c * LR, LR), :].astype(F32)
            mean = jnp.sum(pace1(_sum(_tiles(x)), (c - c0) / n), axis=-1, keepdims=True) * (1.0 / D)
            mean_b = _rb(mean)
            xc = x - mean_b
            shift = mean - mean_b
            sq = jnp.sum(pace2(_sum(_tiles(xc * xc)), (c - c0) / n), axis=-1, keepdims=True)
            var = jnp.maximum(sq * (1.0 / D) - shift * shift, 0.0)
            sd = _rb(jnp.sqrt(_rb(_rb(var) + EPS)))
            xn = _rb(_rb(xc) * pltpu.reciprocal(sd, full_range=False))
            for j, t in enumerate(_tiles(xn)):
                xn_v[j, pl.ds(c * LR, LR), :] = t
            scores = jnp.where(lane == c, jnp.sum(xn * wr, axis=-1, keepdims=True), scores)
        r_v[...] = scores

    def qkv_tile(i, n):
        dst, off = [(q_v, 0), (k_v, HALO), (v_v, HALO)][n // NJ]
        return dst.at[n % NJ, pl.ds(off + i * T, T)]

    def project(i, p, kts=range(NJ)):
        res = _tiles(_nt(_rows(xn_v, i * T, T, kts), _rows(wt_v, p * D, D, kts)))
        for j, t in enumerate(res):
            dst = qkv_tile(i, p * NJ + j)
            dst[...] = t if kts[0] == 0 else dst[...] + t
            if i == 0 and p != Q:
                (k_v, v_v)[p - K][j, pl.ds(0, HALO), :] = jnp.broadcast_to(t[0:1], (HALO, 128))
        return res

    def project_pieces(i):
        for n0 in range(0, 3 * NJ, 4):
            ns = range(n0, min(n0 + 4, 3 * NJ))
            part = _nt(_rows(xn_v, i * T, T, LAST), _rows(wt_v, n0 * 128, len(ns) * 128, LAST))
            yield []
            for n, t in zip(ns, _tiles(part)):
                res = t + _nt(_rows(xn_v, i * T, T, FIRST), _rows(wt_v, n * 128, 128, FIRST))
                qkv_tile(i, n)[...] = res
                yield [res]

    def attention(c0, n, pace):
        for c in range(c0, c0 + n):
            r0 = c * AR
            q = [q_v[j, pl.ds(r0, AR), :] for j in range(NJ)]
            ls = [pace(_sum([q[j] * k_v[j, pl.ds(HALO + r0 - DIL * w, AR), :] for j in range(NJ)]),
                       (c - c0 + w / W) / n) for w in range(W)]
            ls = [a + pltpu.roll(a, 2 * H, 1) for a in ls]
            ls = [a + pltpu.roll(a, H, 1) for a in ls]
            for w in range(W):
                if r0 < DIL * w:
                    pos = lax.broadcasted_iota(jnp.int32, (AR, 128), 0) + r0
                    ls[w] = jnp.where(pos >= DIL * w, ls[w], NEG / SCALE)
            mx = jnp.maximum
            top = mx(mx(mx(ls[0], ls[1]), mx(ls[2], ls[3])), mx(mx(ls[4], ls[5]), mx(ls[6], ls[7])))
            es = [jnp.exp2((a - top) * (SCALE * LOG2E)) for a in ls]
            den = _sum(es)
            inv = pltpu.reciprocal(den, approx=True)
            inv = inv * (2.0 - den * inv)
            for j in range(NJ):
                o_v[j, pl.ds(r0, AR), :] = inv * _sum(
                    [es[w] * v_v[j, pl.ds(HALO + r0 - DIL * w, AR), :] for w in range(W)])

    def route():
        r = _rb(r_v[...]) + 0.0
        row = (lax.broadcasted_iota(jnp.int32, (LR, 128), 1) * LR
               + lax.broadcasted_iota(jnp.int32, (LR, 128), 0))
        bits = lax.bitcast_convert_type(r, jnp.int32)
        taken = -2 ** 31
        key = jnp.where(r != r, taken + 1, jnp.where(bits >= 0, bits, bits ^ 0x7FFFFFFF))
        sub = lax.broadcasted_iota(jnp.int32, (8, D), 0)
        xs = jnp.zeros((8, D), F32)
        score = jnp.zeros((8, D), F32)
        picks = []
        for n in range(2):
            hit = jnp.min(jnp.where(key == jnp.max(key, keepdims=True), row, S - 1), keepdims=True)
            key = jnp.where(row == hit, taken, key)
            picks.append(jnp.clip(hit[0, 0], 0, S - 1))
            xs = jnp.where(sub == n, _rows(xn_v, picks[n], 1), xs)
            score = jnp.where(sub == n, jnp.sum(jnp.where(row == hit, r, 0.0), keepdims=True), score)
        return picks, xs, score

    def routed_pieces(result):
        head, rest = pl.ds(0, D - 128), pl.ds(D - 128, 128)
        picks, xs, score = route()
        for _ in range(FFN_DELAY):
            yield
        xa, xb = xs[:, :D - 128], xs[:, D - 128:]
        hidden = []
        for f0 in range(0, F, 512):
            nf = min(512, F - f0)
            gb = _nt(xb, wg_v[pl.ds(f0, nf), rest])
            if nf == 512:
                yield
            ub = _nt(xb, wu_v[pl.ds(f0, nf), rest])
            yield
            hs = []
            for c in range(0, nf, 128):
                nc = min(128, nf - c)
                g = _rb(gb[:, c:c + nc] + _nt(xa, wg_v[pl.ds(f0 + c, nc), head]))
                yield
                u = _rb(ub[:, c:c + nc] + _nt(xa, wu_v[pl.ds(f0 + c, nc), head]))
                hs.append(_rb(_rb(_silu(g)) * u))
                yield
            hidden.append((f0, nf, hs))
        ya, yb = jnp.zeros((8, D - 128), F32), jnp.zeros((8, 128), F32)
        for f0, nf, hs in hidden:
            for c, h in enumerate(hs):
                ya += _nn(h, wd_v[pl.ds(f0 + c * 128, h.shape[1]), head])
                yield
            yb += _nn(jnp.concatenate(hs, axis=1), wd_v[pl.ds(f0, nf), rest])
            yield
        y = _rb(jnp.concatenate([ya, yb], axis=1))
        result.extend([picks, _rb(y * _rb(jax.nn.sigmoid(score)))])

    def output(r0, n):
        s = _nn(_rows(o_v, r0, n), _rows(wop_v, 0, D))
        for c in range(0, n, LR):
            x = x_v[pl.ds(r0 + c, LR), :].astype(F32)
            out_v[pl.ds(r0 + c, LR), :] = (x + s[c:c + LR] * _silu(_rows(xn_v, r0 + c, LR))).astype(BF16)
        return _tiles(s)

    done = {"attention": 0, "layernorm": T // LR}

    def side_work(pacer, na, nl, leads):
        attention(done["attention"], na, pacer.at(leads[0]))
        layernorm(done["layernorm"], nl, pacer.at(leads[1]), pacer.at(leads[2]))
        done["attention"] += na
        done["layernorm"] += nl

    def project_region(plan, leads, kts=range(NJ)):
        pacer = new_pacer()
        for i, p, na, nl in plan:
            pacer.add(project(i, p, kts))
            side_work(pacer, na, nl, leads)

    def routed_region(plan, leads):
        pacer, result = new_pacer(), []
        routed = routed_pieces(result)
        res, unit = [], 0
        for i in range(5, S // T):
            for piece in project_pieces(i):
                next(routed, None)
                res += piece
                if len(res) == NJ:
                    pacer.add(res)
                    side_work(pacer, plan[unit], 0, leads)
                    if WO_FIRST <= unit < WO_FIRST + NJ:
                        prep_wo(unit - WO_FIRST, pacer.at(0))
                    res, unit = [], unit + 1
        for _ in routed:
            pass
        picks, update = result
        for n, idx in enumerate(picks):
            for j, t in enumerate(_tiles(update[n:n + 1])):
                xn_v[j, pl.ds(idx, 1), :] = _rb(xn_v[j, pl.ds(idx, 1), :] + t)

    def output_region(plan, leads):
        pacer = new_pacer()
        for n, block in enumerate(OUT_BLOCKS):
            pacer.add(output(*block))
            out_copy(n).start()
            if n < len(plan):
                side_work(pacer, plan[n], 0, leads)

    for copy in (wr_copy(), x_copy(0), wq_copy(0), x_copy(1), wq_copy(1), wkv_copy(K), wkv_copy(V),
                 x_copy(2), x_copy(3), wo_copy()):
        copy.start()
    r_v[...] = jnp.zeros_like(r_v)
    wr_copy().wait()
    x_copy(0).wait()
    layernorm(0, T // LR)
    wq_copy(0).wait()
    prep_wqkv(Q, range(KA))
    x_copy(1).wait()
    project_region(*PLAN_FIRST, range(KA))
    wq_copy(1).wait()
    prep_wqkv(Q, range(KA, NJ))
    project(1, Q, range(KA))
    project(0, Q, range(KA, NJ))
    wkv_copy(K).wait()
    prep_wqkv(K)
    project(1, Q, range(KA, NJ))
    project(0, K)
    x_copy(2).wait()
    wkv_copy(V).wait()
    prep_wqkv(V)
    project_region(*PLAN0)

    x_copy(3).wait()
    for copy in ffn_copies():
        copy.start()
    project_region(*PLAN1)
    wo_copy().wait()
    fence().start()
    project_region(*PLAN2)
    for copy in ffn_copies():
        copy.wait()
    routed_region(*PLAN3)
    fence().wait()
    output_region(*PLAN4)
    for n in range(len(OUT_BLOCKS)):
        out_copy(n).wait()
    assert done == {"attention": S // AR, "layernorm": S // LR}


@jax.jit
def pallas_recurrent_scan__sliding_local_dilated__moe_arch_mod__prompt_kernel(
    A_x: jax.Array,
    A_wqkv: jax.Array,
    A_wo: jax.Array,
    B_x: jax.Array,
    B_w_r: jax.Array,
    B_w_gate: jax.Array,
    B_w_up: jax.Array,
    B_w_down: jax.Array,
):
    del B_x
    hbm = pl.BlockSpec(memory_space=pltpu.HBM)
    vmem = pltpu.VMEM
    dma = pltpu.SemaphoreType.DMA
    out = pl.pallas_call(
        _kernel,
        out_shape=jax.ShapeDtypeStruct((S, D), BF16),
        in_specs=[hbm] * 7,
        out_specs=hbm,
        scratch_shapes=[
            vmem((S, D), BF16),
            vmem((NJ, S, 128), F32),
            vmem((NJ, S, 128), F32),
            vmem((NJ, HALO + S, 128), F32),
            vmem((NJ, HALO + S, 128), F32),
            vmem((NJ, S, 128), F32),
            vmem((S, D), BF16),
            vmem((D,), BF16),
            vmem((D,), BF16),
            vmem((3, D, D), BF16),
            vmem((NJ, 3 * D // 2, 128), U32),
            vmem((D, D), BF16),
            vmem((NJ, D // 2, 128), U32),
            vmem((F, D), BF16),
            vmem((F, D), BF16),
            vmem((F, D), BF16),
            vmem((NJ, D // 2, 128), U32),
            vmem((LR, 128), F32),
            dma((14,)), dma((len(OUT_BLOCKS),)),
        ],
        compiler_params=pltpu.CompilerParams(vmem_limit_bytes=64 * 1024 * 1024),
    )(A_x.reshape(S, D), A_wqkv, A_wo, B_w_r, B_w_gate.T, B_w_up.T, B_w_down)
    return out.reshape(1, S, D)
```

```python
import numpy as np
import jax
import jax.numpy as jnp
from jax import lax
import jax.experimental.pallas as pl
import jax.experimental.pallas.tpu as pltpu

S, D, H, W, DIL, F = 2048, 640, 32, 8, 2, 1728
DH = D // H
NJ = D // 128
T = 256
HALO = 16
LR = 16
AR = 8
F32, BF16, U32 = jnp.float32, jnp.bfloat16, jnp.uint32
EPS = 1.00135803e-05
NEG = -999292928.0
SCALE = DH ** -0.5
LOG2E = 1.4426950408889634
LOW, HIGH = np.uint32(0xFFFF), np.uint32(0xFFFF0000)
Q, K, V = 0, 1, 2
FIRST, LAST = range(NJ - 1), [NJ - 1]

KA = 2
X_BLOCKS = [(0, T), (T, T), (2 * T, 2 * T), (4 * T, 4 * T)]
WQ_BLOCKS = [(0, KA * 128), (KA * 128, D - KA * 128)]
OUT_BLOCKS = [(i * T, T) for i in range(7)] + [(7 * T, 128), (7 * T + 128, 96), (7 * T + 224, 32)]

PLAN_FIRST = [(0, Q, 0, 16)], (0, 50, 15)
PLAN0 = [(1, K, 0, 16), (0, V, 0, 12)], (0, 12, 7)
PLAN1 = [(1, V, 8, 8), (2, Q, 7, 8), (2, K, 7, 7), (2, V, 6, 5)], (10, 10, 6)
PLAN2 = [(3, Q, 9, 8), (3, K, 8, 7), (3, V, 8, 7), (4, Q, 9, 7), (4, K, 9, 7), (4, V, 7, 4)], (15, 15, 10)
PLAN3 = [13, 11, 11, 11, 10, 10, 10, 11, 10], (10, 0, 0)
PLAN4 = [12, 12, 12, 12, 12, 13, 8], (15, 0, 0)
FFN_DELAY = 4
WO_FIRST = 3


def _rb(x):
    return x.astype(BF16).astype(F32)


def _silu(z):
    h = 0.5 * z
    return h + h * jnp.tanh(h)


def _sum(terms):
    total = terms[0]
    for t in terms[1:]:
        total = total + t
    return total


def _tiles(x):
    return [x[:, j * 128:(j + 1) * 128] for j in range(x.shape[1] // 128)]


def _rows(ref, r0, n, js=range(NJ)):
    if ref.dtype == U32:
        return jnp.concatenate([pltpu.bitcast(ref[j, pl.ds(r0 // 2, n // 2), :], BF16) for j in js], axis=1)
    return jnp.concatenate([ref[j, pl.ds(r0, n), :] for j in js], axis=1)


def _nn(a, b):
    return jnp.dot(a, b, preferred_element_type=F32)


def _nt(a, b):
    return lax.dot_general(a, b, (((1,), (1,)), ((), ())), preferred_element_type=F32)


def _no_pace(x, frac):
    return x


class Pacer:
    def __init__(self, keep):
        self.keep = keep
        self.tiles = []
        self.start = 0

    def add(self, tiles):
        self.start = len(self.tiles)
        self.tiles += tiles

    def at(self, lead):
        def pace(x, frac):
            pos = self.start + frac * (len(self.tiles) - self.start) - lead / 10
            if pos < 0:
                return x
            tile = self.tiles[min(int(pos), len(self.tiles) - 1)]
            r0 = int(pos % 1 * tile.shape[0]) // AR * AR
            late = tile[r0:r0 + AR]
            if late.dtype != x.dtype:
                late = lax.bitcast_convert_type(late, x.dtype)
            return jnp.concatenate([jnp.where(self.keep, x[r:r + AR], late)
                                    for r in range(0, x.shape[0], AR)], axis=0)
        return pace


def _kernel(x_hbm, wqkv_hbm, wo_hbm, wr_hbm, wg_hbm, wu_hbm, wd_hbm, out_hbm,
            x_v, xn_v, q_v, k_v, v_v, o_v, out_v, wr_v, fence_v, wqkv_v, wt_v, wo_v, wop_v, wg_v, wu_v, wd_v,
            tmp_v, r_v, sem_in, sem_out):
    def x_copy(n):
        rows = pl.ds(*X_BLOCKS[n])
        return pltpu.make_async_copy(x_hbm.at[rows], x_v.at[rows], sem_in.at[n])

    def wq_copy(n):
        rows = pl.ds(*WQ_BLOCKS[n])
        return pltpu.make_async_copy(wqkv_hbm.at[rows, pl.ds(0, D)], wqkv_v.at[Q, rows], sem_in.at[4 + n])

    def wkv_copy(p):
        return pltpu.make_async_copy(wqkv_hbm.at[:, pl.ds(p * D, D)], wqkv_v.at[p], sem_in.at[5 + p])

    def wo_copy():
        return pltpu.make_async_copy(wo_hbm, wo_v, sem_in.at[8])

    def wr_copy():
        return pltpu.make_async_copy(wr_hbm, wr_v, sem_in.at[9])

    def fence():
        return pltpu.make_async_copy(wr_hbm, fence_v, sem_in.at[10])

    def ffn_copies():
        return [pltpu.make_async_copy(src, dst, sem_in.at[11 + m])
                for m, (src, dst) in enumerate(((wg_hbm, wg_v), (wu_hbm, wu_v), (wd_hbm, wd_v)))]

    def out_copy(n):
        rows = pl.ds(*OUT_BLOCKS[n])
        return pltpu.make_async_copy(out_v.at[rows], out_hbm.at[rows], sem_out.at[n])

    def router_weights():
        return wr_v[...].astype(F32).reshape(1, D)

    def new_pacer():
        bits = lax.bitcast_convert_type(router_weights()[:, :128], jnp.int32)
        return Pacer(jnp.broadcast_to(bits | 1, (AR, 128)) != 0)

    def regroup(src, dst, row0):
        for dd in range(DH // 2):
            even = src[pl.ds(dd, H // 2, stride=DH), :]
            odd = src[pl.ds(dd + DH // 2, H // 2, stride=DH), :]
            r = (row0 + 2 * dd * H) // 2
            dst[pl.ds(r, H // 2), :] = (even & LOW) | (odd << 16)
            dst[pl.ds(r + H // 2, H // 2), :] = (even >> 16) | (odd & HIGH)

    def prep_wqkv(p, kts=range(NJ)):
        for kt in kts:
            tmp_v[kt] = pltpu.bitcast(wqkv_v[p, pl.ds(kt * 128, 128), :].T, U32)
        for kt in kts:
            regroup(tmp_v.at[kt], wt_v.at[kt], p * D)

    def prep_wo(j, pace):
        for r in range(0, D, 64):
            words = pltpu.bitcast(wo_v[pl.ds(r, 64), pl.ds(j * 128, 128)], U32)
            tmp_v[j, pl.ds(r // 2, 32), :] = pace(words, r / D / 2)
        regroup(tmp_v.at[j], wop_v.at[j], 0)

    def layernorm(c0, n, pace1=_no_pace, pace2=_no_pace):
        if n == 0:
            return
        wr = router_weights()
        lane = lax.broadcasted_iota(jnp.int32, (LR, 128), 1)
        scores = r_v[...]
        for c in range(c0, c0 + n):
            x = x_v[pl.ds(c * LR, LR), :].astype(F32)
            mean = jnp.sum(pace1(_sum(_tiles(x)), (c - c0) / n), axis=-1, keepdims=True) * (1.0 / D)
            mean_b = _rb(mean)
            xc = x - mean_b
            shift = mean - mean_b
            sq = jnp.sum(pace2(_sum(_tiles(xc * xc)), (c - c0) / n), axis=-1, keepdims=True)
            var = jnp.maximum(sq * (1.0 / D) - shift * shift, 0.0)
            sd = _rb(jnp.sqrt(_rb(_rb(var) + EPS)))
            xn = _rb(_rb(xc) * pltpu.reciprocal(sd, full_range=False))
            for j, t in enumerate(_tiles(xn)):
                xn_v[j, pl.ds(c * LR, LR), :] = t
            scores = jnp.where(lane == c, jnp.sum(xn * wr, axis=-1, keepdims=True), scores)
        r_v[...] = scores

    def qkv_tile(i, n):
        dst, off = [(q_v, 0), (k_v, HALO), (v_v, HALO)][n // NJ]
        return dst.at[n % NJ, pl.ds(off + i * T, T)]

    def project(i, p, kts=range(NJ)):
        res = _tiles(_nt(_rows(xn_v, i * T, T, kts), _rows(wt_v, p * D, D, kts)))
        for j, t in enumerate(res):
            dst = qkv_tile(i, p * NJ + j)
            dst[...] = t if kts[0] == 0 else dst[...] + t
            if i == 0 and p != Q:
                (k_v, v_v)[p - K][j, pl.ds(0, HALO), :] = jnp.broadcast_to(t[0:1], (HALO, 128))
        return res

    def project_pieces(i):
        for n0 in range(0, 3 * NJ, 4):
            ns = range(n0, min(n0 + 4, 3 * NJ))
            part = _nt(_rows(xn_v, i * T, T, LAST), _rows(wt_v, n0 * 128, len(ns) * 128, LAST))
            yield []
            for n, t in zip(ns, _tiles(part)):
                res = t + _nt(_rows(xn_v, i * T, T, FIRST), _rows(wt_v, n * 128, 128, FIRST))
                qkv_tile(i, n)[...] = res
                yield [res]

    def attention(c0, n, pace):
        for c in range(c0, c0 + n):
            r0 = c * AR
            q = [q_v[j, pl.ds(r0, AR), :] for j in range(NJ)]
            ls = [pace(_sum([q[j] * k_v[j, pl.ds(HALO + r0 - DIL * w, AR), :] for j in range(NJ)]),
                       (c - c0 + w / W) / n) for w in range(W)]
            ls = [a + pltpu.roll(a, 2 * H, 1) for a in ls]
            ls = [a + pltpu.roll(a, H, 1) for a in ls]
            for w in range(W):
                if r0 < DIL * w:
                    pos = lax.broadcasted_iota(jnp.int32, (AR, 128), 0) + r0
                    ls[w] = jnp.where(pos >= DIL * w, ls[w], NEG / SCALE)
            mx = jnp.maximum
            top = mx(mx(mx(ls[0], ls[1]), mx(ls[2], ls[3])), mx(mx(ls[4], ls[5]), mx(ls[6], ls[7])))
            es = [jnp.exp2((a - top) * (SCALE * LOG2E)) for a in ls]
            den = _sum(es)
            inv = pltpu.reciprocal(den, approx=True)
            inv = inv * (2.0 - den * inv)
            for j in range(NJ):
                o_v[j, pl.ds(r0, AR), :] = inv * _sum(
                    [es[w] * v_v[j, pl.ds(HALO + r0 - DIL * w, AR), :] for w in range(W)])

    def route():
        r = _rb(r_v[...])
        r = jnp.where(r == 0.0, 0.0, r)
        row = (lax.broadcasted_iota(jnp.int32, (LR, 128), 1) * LR
               + lax.broadcasted_iota(jnp.int32, (LR, 128), 0))
        bits = lax.bitcast_convert_type(r, jnp.int32)
        taken = -2 ** 31
        key = jnp.where(r != r, taken + 1, jnp.where(bits >= 0, bits, bits ^ 0x7FFFFFFF))
        sub = lax.broadcasted_iota(jnp.int32, (8, D), 0)
        xs = jnp.zeros((8, D), F32)
        score = jnp.zeros((8, D), F32)
        picks = []
        for n in range(2):
            hit = jnp.min(jnp.where(key == jnp.max(key, keepdims=True), row, S - 1), keepdims=True)
            key = jnp.where(row == hit, taken, key)
            picks.append(jnp.clip(hit[0, 0], 0, S - 1))
            xs = jnp.where(sub == n, _rows(xn_v, picks[n], 1), xs)
            score = jnp.where(sub == n, jnp.sum(jnp.where(row == hit, r, 0.0), keepdims=True), score)
        return picks, xs, score

    def routed_pieces(result):
        head, rest = pl.ds(0, D - 128), pl.ds(D - 128, 128)
        picks, xs, score = route()
        for _ in range(FFN_DELAY):
            yield
        xa, xb = xs[:, :D - 128], xs[:, D - 128:]
        hidden = []
        for f0 in range(0, F, 512):
            nf = min(512, F - f0)
            gb = _nt(xb, wg_v[pl.ds(f0, nf), rest])
            if nf == 512:
                yield
            ub = _nt(xb, wu_v[pl.ds(f0, nf), rest])
            yield
            hs = []
            for c in range(0, nf, 128):
                nc = min(128, nf - c)
                g = _rb(gb[:, c:c + nc] + _nt(xa, wg_v[pl.ds(f0 + c, nc), head]))
                yield
                u = _rb(ub[:, c:c + nc] + _nt(xa, wu_v[pl.ds(f0 + c, nc), head]))
                hs.append(_rb(_rb(_silu(g)) * u))
                yield
            hidden.append((f0, nf, hs))
        ya, yb = jnp.zeros((8, D - 128), F32), jnp.zeros((8, 128), F32)
        for f0, nf, hs in hidden:
            for c, h in enumerate(hs):
                ya += _nn(h, wd_v[pl.ds(f0 + c * 128, h.shape[1]), head])
                yield
            yb += _nn(jnp.concatenate(hs, axis=1), wd_v[pl.ds(f0, nf), rest])
            yield
        y = _rb(jnp.concatenate([ya, yb], axis=1))
        result.extend([picks, _rb(y * _rb(jax.nn.sigmoid(score)))])

    def output(r0, n):
        s = _nn(_rows(o_v, r0, n), _rows(wop_v, 0, D))
        for c in range(0, n, LR):
            x = x_v[pl.ds(r0 + c, LR), :].astype(F32)
            out_v[pl.ds(r0 + c, LR), :] = (x + s[c:c + LR] * _silu(_rows(xn_v, r0 + c, LR))).astype(BF16)
        return _tiles(s)

    done = {"attention": 0, "layernorm": T // LR}

    def side_work(pacer, na, nl, leads):
        attention(done["attention"], na, pacer.at(leads[0]))
        layernorm(done["layernorm"], nl, pacer.at(leads[1]), pacer.at(leads[2]))
        done["attention"] += na
        done["layernorm"] += nl

    def project_region(plan, leads, kts=range(NJ)):
        pacer = new_pacer()
        for i, p, na, nl in plan:
            pacer.add(project(i, p, kts))
            side_work(pacer, na, nl, leads)

    def routed_region(plan, leads):
        pacer, result = new_pacer(), []
        routed = routed_pieces(result)
        res, unit = [], 0
        for i in range(5, S // T):
            for piece in project_pieces(i):
                next(routed, None)
                res += piece
                if len(res) == NJ:
                    pacer.add(res)
                    side_work(pacer, plan[unit], 0, leads)
                    if WO_FIRST <= unit < WO_FIRST + NJ:
                        prep_wo(unit - WO_FIRST, pacer.at(0))
                    res, unit = [], unit + 1
        for _ in routed:
            pass
        picks, update = result
        for n, idx in enumerate(picks):
            for j, t in enumerate(_tiles(update[n:n + 1])):
                xn_v[j, pl.ds(idx, 1), :] = _rb(xn_v[j, pl.ds(idx, 1), :] + t)

    def output_region(plan, leads):
        pacer = new_pacer()
        for n, block in enumerate(OUT_BLOCKS):
            pacer.add(output(*block))
            out_copy(n).start()
            if n < len(plan):
                side_work(pacer, plan[n], 0, leads)

    for copy in (wr_copy(), x_copy(0), wq_copy(0), x_copy(1), wq_copy(1), wkv_copy(K), wkv_copy(V),
                 x_copy(2), x_copy(3), wo_copy()):
        copy.start()
    r_v[...] = jnp.zeros_like(r_v)
    wr_copy().wait()
    x_copy(0).wait()
    layernorm(0, T // LR)
    wq_copy(0).wait()
    prep_wqkv(Q, range(KA))
    x_copy(1).wait()
    project_region(*PLAN_FIRST, range(KA))
    wq_copy(1).wait()
    prep_wqkv(Q, range(KA, NJ))
    project(1, Q, range(KA))
    project(0, Q, range(KA, NJ))
    wkv_copy(K).wait()
    prep_wqkv(K)
    project(1, Q, range(KA, NJ))
    project(0, K)
    x_copy(2).wait()
    wkv_copy(V).wait()
    prep_wqkv(V)
    project_region(*PLAN0)

    x_copy(3).wait()
    for copy in ffn_copies():
        copy.start()
    project_region(*PLAN1)
    wo_copy().wait()
    fence().start()
    project_region(*PLAN2)
    for copy in ffn_copies():
        copy.wait()
    routed_region(*PLAN3)
    fence().wait()
    output_region(*PLAN4)
    for n in range(len(OUT_BLOCKS)):
        out_copy(n).wait()
    assert done == {"attention": S // AR, "layernorm": S // LR}


@jax.jit
def pallas_recurrent_scan__sliding_local_dilated__moe_arch_mod__prompt_kernel(
    A_x: jax.Array,
    A_wqkv: jax.Array,
    A_wo: jax.Array,
    B_x: jax.Array,
    B_w_r: jax.Array,
    B_w_gate: jax.Array,
    B_w_up: jax.Array,
    B_w_down: jax.Array,
):
    del B_x
    hbm = pl.BlockSpec(memory_space=pltpu.HBM)
    vmem = pltpu.VMEM
    dma = pltpu.SemaphoreType.DMA
    out = pl.pallas_call(
        _kernel,
        out_shape=jax.ShapeDtypeStruct((S, D), BF16),
        in_specs=[hbm] * 7,
        out_specs=hbm,
        scratch_shapes=[
            vmem((S, D), BF16),
            vmem((NJ, S, 128), F32),
            vmem((NJ, S, 128), F32),
            vmem((NJ, HALO + S, 128), F32),
            vmem((NJ, HALO + S, 128), F32),
            vmem((NJ, S, 128), F32),
            vmem((S, D), BF16),
            vmem((D,), BF16),
            vmem((D,), BF16),
            vmem((3, D, D), BF16),
            vmem((NJ, 3 * D // 2, 128), U32),
            vmem((D, D), BF16),
            vmem((NJ, D // 2, 128), U32),
            vmem((F, D), BF16),
            vmem((F, D), BF16),
            vmem((F, D), BF16),
            vmem((NJ, D // 2, 128), U32),
            vmem((LR, 128), F32),
            dma((14,)), dma((len(OUT_BLOCKS),)),
        ],
        compiler_params=pltpu.CompilerParams(vmem_limit_bytes=64 * 1024 * 1024),
    )(A_x.reshape(S, D), A_wqkv, A_wo, B_w_r, B_w_gate.T, B_w_up.T, B_w_down)
    return out.reshape(1, S, D)
```
